```python
import jax
import jax.numpy as jnp

def _softmax(x, axis=-1):
    return jax.nn.softmax(x, axis=axis)
def _gelu(x):
    return jax.nn.gelu(x, approximate=True)
def _silu(x):
    return jax.nn.silu(x)
def _sigmoid(x):
    return jax.nn.sigmoid(x)
def _layernorm(x, axis=-1, eps=1e-5):
    m = jnp.mean(x, axis=axis, keepdims=True)
    v = jnp.var(x, axis=axis, keepdims=True)
    return (x - m) / jnp.sqrt(v + eps)
def _scatter_add(tgt, idx, src, axis=0):
    return tgt.at[idx].add(src)
def _segment_sum(src, seg, n):
    return jax.ops.segment_sum(src, seg, n)
class _Rng:
    def __init__(self, key):
        self._k = key
    def _next(self):
        self._k, sub = jax.random.split(self._k)
        return sub
    def normal(self, shape):
        return jax.random.normal(self._next(), shape, dtype=jnp.bfloat16)
    def randint(self, lo, hi, shape):
        return jax.random.randint(self._next(), shape, lo, hi, dtype=jnp.int32)
    def uniform(self, shape, lo=0.0, hi=1.0):
        return jax.random.uniform(self._next(), shape, jnp.bfloat16, lo, hi)
    def permutation(self, n):
        return jax.random.permutation(self._next(), n)


kernel_name = 'interleave_layers__grouped_kv_mqa__sliding_local_dilated__prompt'

def setup_inputs():
    _rng = _Rng(jax.random.key(int.from_bytes(__import__("os").urandom(4), "little")))
    _w = (lambda a: (lambda t: t.astype(jnp.bfloat16) if jnp.issubdtype(t.dtype, jnp.floating) else t)(jnp.asarray(a)))
    def _A_setup():
        B, S, D, H = 1, 2048, 1024, 32
        Dh = D // H
        return {
            "x": _w((lambda *s: _rng.normal(s) * 0.05)(B, S, D)),
            "wq": _w((lambda *s: _rng.normal(s) * 0.05)(D, H * Dh)),
            "wk": _w((lambda *s: _rng.normal(s) * 0.05)(D, Dh)),
            "wv": _w((lambda *s: _rng.normal(s) * 0.05)(D, Dh)),
            "wo": _w((lambda *s: _rng.normal(s) * 0.05)(H * Dh, D)),
        }
    _A_in = _A_setup()

    def _B_setup():
        B, S, D = 1, 2048, 1024
        return {
            "x": _w((lambda *s: _rng.normal(s) * 0.05)(B, S, D)),
            "wqkv": _w((lambda *s: _rng.normal(s) * 0.05)(D, 3 * D)),
            "wo": _w((lambda *s: _rng.normal(s) * 0.05)(D, D)),
        }
    _B_in = _B_setup()

    return {
        "A_x": _A_in["x"],
        "A_wq": _A_in["wq"],
        "A_wk": _A_in["wk"],
        "A_wv": _A_in["wv"],
        "A_wo": _A_in["wo"],
        "B_x": _B_in["x"],
        "B_wqkv": _B_in["wqkv"],
        "B_wo": _B_in["wo"],
    }

def reference(A_x, A_wq, A_wk, A_wv, A_wo, B_x, B_wqkv, B_wo):
    def _A_ref(x, wq, wk, wv, wo):
        B, S, D = x.shape
        H = 32
        Dh = D // H
        q = (lambda x, *d: x.transpose(*d))((x @ wq).reshape(B, S, H, Dh), 0, 2, 1, 3)
        k = x @ wk
        v = x @ wv
        scores = jnp.einsum("bhqd,bkd->bhqk", q, k) * (Dh ** -0.5)
        p = _softmax(scores, axis=-1)
        o = jnp.einsum("bhqk,bkd->bhqd", p, v)
        return (lambda x, *d: x.transpose(*d))(o, 0, 2, 1, 3).reshape(B, S, H * Dh) @ wo

    def _B_ref(x, wqkv, wo):
        B, S, D = x.shape
        H = 32; Dh = D // H
        W, dil = 8, 2
        qkv = (lambda x, *d: x.transpose(*d))((x @ wqkv).reshape(B, S, 3, H, Dh), 2, 0, 3, 1, 4)
        q, k, v = qkv[0], qkv[1], qkv[2]
        scale = Dh ** -0.5
        pos = jnp.arange(S)
        off = jnp.arange(W) * dil
        idx = pos[:, None] - off[None, :]
        mask = idx >= 0
        idx_c = jnp.where(mask, idx, 0).reshape(-1)
        kg = k[:, :, idx_c, :].reshape(B, H, S, W, Dh)
        vg = v[:, :, idx_c, :].reshape(B, H, S, W, Dh)
        logits = jnp.einsum("bhsd,bhswd->bhsw", q, kg) * scale
        logits = jnp.where(mask[None, None, :, :], logits, -1e9)
        attn = _softmax(logits, axis=-1)
        o = jnp.einsum("bhsw,bhswd->bhsd", attn, vg)
        return (lambda x, *d: x.transpose(*d))(o, 0, 2, 1, 3).reshape(B, S, D) @ wo

    x = A_x
    x = x + _A_ref(_layernorm(x, axis=-1), A_wq, A_wk, A_wv, A_wo)
    x = x + _B_ref(_layernorm(x, axis=-1), B_wqkv, B_wo)
    x = x + _A_ref(_layernorm(x, axis=-1), A_wq, A_wk, A_wv, A_wo)
    x = x + _B_ref(_layernorm(x, axis=-1), B_wqkv, B_wo)
    return x
```

```python
import functools
import math

import jax
import jax.numpy as jnp
import numpy as np
from jax import lax
from jax.experimental import pallas as pl
from jax.experimental.pallas import tpu as pltpu

F32 = jnp.float32
BF16 = jnp.bfloat16
U32 = jnp.uint32

H = 32
DH = 32
W = 8
DIL = 2
HALO = 16
EPS = 1e-5
LOG2E = math.log2(math.e)

R = 512
SUB = 256
CH = 256
HU = 4
PAD = 33

NT = (((1,), (1,)), ((), ()))
TN = (((0,), (0,)), ((), ()))


def _layernorm(x):
    m = jnp.mean(x, axis=-1, keepdims=True)
    d = x - m
    v = jnp.mean(d * d, axis=-1, keepdims=True)
    return d * lax.rsqrt(v + EPS)


def _kernel(
    x_hbm, wq_hbm, wk_hbm, wv_hbm, woa_hbm, wqkv_hbm, wob_hbm,
    o_ref,
    xin, wq, wk, wv, woa, wqkv, wob,
    wt, wqkv_p, wob_p, tmp,
    xs, ln3, qt, kt, vt_next, kb, vt, ot, lq, lk, lv,
    sems,
):
    S, D = xs.shape
    NB = S // R
    NTILE = D // 128
    step = pl.program_id(0)

    def x_copy(b):
        rows = pl.ds(b * R, R)
        return pltpu.make_async_copy(x_hbm.at[rows], xin.at[rows], sems.at[b])

    w_copies = [
        pltpu.make_async_copy(src, dst, sems.at[NB + i])
        for i, (src, dst) in enumerate(
            [(wq_hbm, wq), (wk_hbm, wk), (wv_hbm, wv), (woa_hbm, woa),
             (wqkv_hbm, wqkv), (wob_hbm, wob)]
        )
    ]

    @pl.when(step == 0)
    def _():
        for c in w_copies[:3]:
            c.start()
        for b in range(NB):
            x_copy(b).start()
        for c in w_copies[3:]:
            c.start()
        lk[:, R:, :] = jnp.zeros((NTILE, HALO, 128), F32)
        lv[:, R:, :] = jnp.zeros((NTILE, HALO, 128), F32)
        for c in w_copies[:3]:
            c.wait()
        for j in range(NTILE):
            cols = slice(j * 128, (j + 1) * 128)
            wt[cols, :] = wq[:, cols].T
        wt[D:D + DH, :] = wk[...]
        wt[D + DH:D + 2 * DH, :] = wv[...]

    is_pre = step < NB
    idx = jnp.maximum(step - NB, 0)
    layer = idx // NB
    blk = jnp.where(is_pre, step, idx % NB)
    row0 = pl.multiple_of(blk * R, R)

    @pl.when(is_pre)
    def _():
        x_copy(step).wait()
        for i in range(R // 64):
            rows = pl.ds(row0 + i * 64, 64)
            x = xin[rows, :].astype(F32)
            xs[rows, :] = x
            ln3[i * 64:(i + 1) * 64, :] = _layernorm(x).astype(BF16)

    @pl.when(step == NB)
    def _():
        for c in w_copies[3:]:
            c.wait()
        nrc = D // 256

        def permute_cols(n, _):
            part = n // nrc
            rows = pl.ds(pl.multiple_of((n % nrc) * 256, 256), 256)
            for g in range(NTILE):
                cols = pl.ds(pl.multiple_of(part * D + g * 128, 128), 128)
                t = pltpu.bitcast(wqkv[rows, cols], U32).T
                for hl in range(4):
                    tmp[pl.ds((4 * g + hl) * PAD, DH), :] = t[hl * DH:(hl + 1) * DH]
            for g in range(NTILE):
                cols = pl.ds(pl.multiple_of(part * D + g * 128, 128), 128)
                t = jnp.concatenate(
                    [tmp[pl.ds(4 * g + dl, H, stride=PAD), :] for dl in range(4)], axis=0
                )
                wqkv_p[rows, cols] = pltpu.bitcast(t.T, BF16)

        lax.fori_loop(0, 3 * nrc, permute_cols, None)

        def permute_rows(j, _):
            cols = pl.ds(pl.multiple_of(j * 128, 128), 128)
            for i in range(H // 2):
                tmp[pl.ds(i * PAD, DH), :] = pltpu.bitcast(
                    wob[i * 2 * DH:(i + 1) * 2 * DH, cols], U32
                )
            for e in range(DH // 2):
                a = tmp[pl.ds(e, H // 2, stride=PAD), :]
                b = tmp[pl.ds(DH // 2 + e, H // 2, stride=PAD), :]
                even = (a & np.uint32(0xFFFF)) | (b << 16)
                odd = (a >> 16) | (b & np.uint32(0xFFFF0000))
                wob_p[e * 2 * H:(e + 1) * 2 * H, cols] = pltpu.bitcast(
                    jnp.concatenate([even, odd], axis=0), BF16
                )

        lax.fori_loop(0, NTILE, permute_rows, None)

    @pl.when(jnp.logical_and(step >= NB, blk == 0))
    def _():
        k = kt[...]
        k = (k - jnp.mean(k, axis=-1, keepdims=True)) * (DH ** -0.5 * LOG2E)
        zeros = jnp.zeros((128 - DH, 128), F32)
        for j in range(S // 128):
            t = jnp.concatenate([k[:, j * 128:(j + 1) * 128], zeros], axis=0).T
            kb[j * 128:(j + 1) * 128, :] = t.astype(BF16)
        vt[...] = vt_next[...]

    def load_q(h):
        return jnp.concatenate([qt[blk, h], jnp.zeros((128 - DH, R), BF16)], axis=0)

    def head_rows(h):
        return pl.ds(pl.multiple_of(h * DH, DH), DH)

    @pl.when(step >= NB)
    def _():
        nch = S // CH

        def fast_heads(it, ok):
            qs = [load_q(it * HU + u) for u in range(HU)]

            def scores(u, c):
                return jnp.dot(kb[c * CH:(c + 1) * CH, :], qs[u], preferred_element_type=F32)

            s = scores(0, 0)
            for u in range(HU):
                acc = l = None
                for c in range(nch):
                    p = jnp.exp2(s)
                    ps = p.reshape(CH // 8, 8, R).sum(axis=0)
                    l = ps if l is None else l + ps
                    n = u * nch + c + 1
                    if n < HU * nch:
                        s = scores(n // nch, n % nch)
                    pv = jnp.dot(
                        vt[:, c * CH:(c + 1) * CH], p.astype(BF16), preferred_element_type=F32
                    )
                    acc = pv if acc is None else acc + pv
                l = jnp.sum(l, axis=0, keepdims=True)
                ot[head_rows(it * HU + u), :] = (acc * (1.0 / l)).astype(BF16)
                amax = jnp.abs(acc).reshape(DH // 8, 8, R)
                good = jnp.logical_and(l >= 1.0, l < 3e38)
                for i in range(DH // 8):
                    good = jnp.logical_and(good, amax[i] < 3e38)
                ok = jnp.where(good, ok, 0.0)
            return ok

        ok = lax.fori_loop(0, H // HU, fast_heads, jnp.ones((8, R), F32))

        @pl.when(jnp.min(ok) < 1.0)
        def _():
            def safe_head(h, _):
                q = load_q(h)

                def chunk(c, carry):
                    m, l, acc = carry
                    keys = pl.ds(pl.multiple_of(c * 128, 128), 128)
                    s = jnp.dot(kb[keys, :], q, preferred_element_type=F32)
                    m_new = jnp.maximum(m, jnp.max(s, axis=0, keepdims=True))
                    alpha = jnp.exp2(m - m_new)
                    p = jnp.exp2(s - m_new)
                    l = alpha * l + jnp.sum(p, axis=0, keepdims=True)
                    acc = alpha * acc + jnp.dot(
                        vt[:, keys], p.astype(BF16), preferred_element_type=F32
                    )
                    return m_new, l, acc

                init = (
                    jnp.full((1, R), -jnp.inf, F32),
                    jnp.zeros((1, R), F32),
                    jnp.zeros((DH, R), F32),
                )
                _, l, acc = lax.fori_loop(0, S // 128, chunk, init)
                ot[head_rows(h), :] = (acc / l).astype(BF16)

            lax.fori_loop(0, H, safe_head, None)

        first = blk == 0
        nsub = R // SUB

        def rows_of(i):
            return pl.ds(row0 + i * SUB, SUB)

        for i in range(nsub):
            a = lax.dot_general(
                ot[:, i * SUB:(i + 1) * SUB], woa[...], TN, preferred_element_type=F32
            )
            xs[rows_of(i), :] = xs[rows_of(i), :] + a

        for i in range(nsub):
            ln = _layernorm(xs[rows_of(i), :]).astype(BF16)
            qkv = jnp.dot(ln, wqkv_p[...], preferred_element_type=F32)
            dst = slice(HALO + i * SUB, HALO + (i + 1) * SUB)
            for t in range(NTILE):
                cols = slice(t * 128, (t + 1) * 128)
                lq[t, i * SUB:(i + 1) * SUB, :] = qkv[:, cols] * (DH ** -0.5 * LOG2E)
                for part, ref in ((1, lk), (2, lv)):
                    z = qkv[:, part * D + t * 128:part * D + (t + 1) * 128]
                    if i == 0:
                        ref[t, 0:HALO, :] = jnp.where(first, z[0:1, :], ref[t, R:, :])
                    ref[t, dst, :] = z

        for i in range(nsub):
            outs = []
            for r in range(i * SUB, (i + 1) * SUB, 16):
                q = [lq[t, r:r + 16, :] for t in range(NTILE)]
                z = []
                for w in range(W):
                    src = slice(HALO + r - DIL * w, HALO + r - DIL * w + 16)
                    y = q[0] * lk[0, src, :]
                    for t in range(1, NTILE):
                        y = y + q[t] * lk[t, src, :]
                    y = y + pltpu.roll(y, 64, 1)
                    y = y + pltpu.roll(y, 32, 1)
                    if r < DIL * w:
                        pos = row0 + r + lax.broadcasted_iota(jnp.int32, (16, 128), 0)
                        y = jnp.where(pos >= DIL * w, y, -1e9 * LOG2E)
                    z.append(y)
                m = functools.reduce(jnp.maximum, z)
                e = [jnp.exp2(y - m) for y in z]
                inv = 1.0 / functools.reduce(jnp.add, e)
                e = [y * inv for y in e]
                o = []
                for t in range(NTILE):
                    acc = None
                    for w in range(W):
                        src = slice(HALO + r - DIL * w, HALO + r - DIL * w + 16)
                        y = e[w] * lv[t, src, :]
                        acc = y if acc is None else acc + y
                    o.append(acc)
                outs.append(jnp.concatenate(o, axis=1).astype(BF16))
            b = jnp.dot(
                jnp.concatenate(outs, axis=0), wob_p[...], preferred_element_type=F32
            )
            x = xs[rows_of(i), :] + b
            xs[rows_of(i), :] = x
            o_ref[i * SUB:(i + 1) * SUB, :] = x.astype(BF16)
            ln3[i * SUB:(i + 1) * SUB, :] = _layernorm(x).astype(BF16)

    @pl.when(step < 2 * NB)
    def _():
        y = lax.dot_general(wt[...], ln3[...], NT, preferred_element_type=F32)
        qt[blk] = y[:D].astype(BF16).reshape(H, DH, R)
        kt[:, pl.ds(row0, R)] = y[D:D + DH]
        vt_next[:, pl.ds(row0, R)] = y[D + DH:].astype(BF16)


@jax.jit
def pallas_interleave_layers__grouped_kv_mqa__sliding_local_dilated__prompt_kernel(
    A_x: jax.Array,
    A_wq: jax.Array,
    A_wk: jax.Array,
    A_wv: jax.Array,
    A_wo: jax.Array,
    B_x: jax.Array,
    B_wqkv: jax.Array,
    B_wo: jax.Array,
):
    del B_x
    _, S, D = A_x.shape
    NB = S // R
    vmem = pltpu.VMEM
    out = pl.pallas_call(
        _kernel,
        grid=(3 * NB,),
        in_specs=[pl.BlockSpec(memory_space=pl.ANY)] * 7,
        out_specs=pl.BlockSpec((R, D), lambda s: (jnp.maximum(s - 2 * NB, 0), 0)),
        out_shape=jax.ShapeDtypeStruct((S, D), A_x.dtype),
        scratch_shapes=[
            vmem((S, D), BF16),
            vmem((D, D), BF16),
            vmem((DH, D), BF16),
            vmem((DH, D), BF16),
            vmem((D, D), BF16),
            vmem((D, 3 * D), BF16),
            vmem((D, D), BF16),
            vmem((D + 2 * DH, D), BF16),
            vmem((D, 3 * D), BF16),
            vmem((D, D), BF16),
            vmem((H * PAD, 128), U32),
            vmem((S, D), F32),
            vmem((R, D), BF16),
            vmem((NB, H, DH, R), BF16),
            vmem((DH, S), F32),
            vmem((DH, S), BF16),
            vmem((S, 128), BF16),
            vmem((DH, S), BF16),
            vmem((D, R), BF16),
            vmem((D // 128, R, 128), F32),
            vmem((D // 128, HALO + R, 128), F32),
            vmem((D // 128, HALO + R, 128), F32),
            pltpu.SemaphoreType.DMA((NB + 6,)),
        ],
        compiler_params=pltpu.CompilerParams(
            dimension_semantics=("arbitrary",),
            vmem_limit_bytes=110 * 2**20,
        ),
        name="interleave_layers",
    )(A_x.reshape(S, D), A_wq, A_wk.T, A_wv.T, A_wo, B_wqkv, B_wo)
    return out.reshape(1, S, D)
```

```python
import functools
import math

import jax
import jax.numpy as jnp
import numpy as np
from jax import lax
from jax.experimental import pallas as pl
from jax.experimental.pallas import tpu as pltpu

F32 = jnp.float32
BF16 = jnp.bfloat16
U32 = jnp.uint32

H = 32
DH = 32
W = 8
DIL = 2
HALO = 16
EPS = 1e-5
QSCALE = DH ** -0.5 * math.log2(math.e)
MASKED = -1e9 * math.log2(math.e)

R = 512
SUB = 256
CH = 256
VK = 16
MK = CH - VK
GS = 2
HU = 4
UNITS = DH // 16 * R // 128
LR = 16
PAD = 33

NT = (((1,), (1,)), ((), ()))


def _layernorm(xs):
    inv_d = 1.0 / (128 * len(xs))
    m = jnp.sum(functools.reduce(jnp.add, xs), axis=-1, keepdims=True) * inv_d
    ds = [x - m for x in xs]
    v = jnp.sum(functools.reduce(jnp.add, [d * d for d in ds]), axis=-1, keepdims=True) * inv_d
    return ds, lax.rsqrt(v + EPS)


def _pack(x):
    return pltpu.bitcast(x.astype(BF16), U32)


def _unpack(x):
    return pltpu.bitcast(x, BF16)


def _half(rows):
    return slice(rows.start // 2, rows.stop // 2)


def _aligned(index, n):
    return pl.ds(pl.multiple_of(index * n, n), n)


def _dot(a, b):
    return jnp.dot(a, b, preferred_element_type=F32)


def _lanes(tiles):
    return jnp.concatenate(tiles, axis=1)


def _tile(t):
    return slice(t * 128, (t + 1) * 128)


def _in_time_order(y):
    return [y[r:r + 8, 0:128] for r in range(0, y.shape[0], 8)]


def _interleave(mxu, *jobs):
    todo = sorted(
        [(start + (stop - start) * i / len(pieces), j, i, piece)
         for j, (pieces, start, stop) in enumerate(jobs) for i, piece in enumerate(pieces)],
        key=lambda item: item[:3],
    )
    for n, piece in enumerate(mxu):
        results = piece()
        while todo and todo[0][0] < n + 1:
            at, _, _, other = todo.pop(0)
            other(results[int((at - n) * len(results))])
    assert not todo


def _kernel(
    x_hbm, wq_hbm, wk_hbm, wv_hbm, woa_hbm, wqkv_hbm, wob_hbm,
    o_ref,
    xin, raw, wkv, wt, woa, wqkv, wob, tmp_c, tmp_r,
    xs, x1, ln, qt, kmean, kb, kv, vt, qb, p0, l0, ot, oa, ob,
    lqk0, lqk1, lv0, lv1, lp0, lp1,
    sems,
):
    T, S, _ = xs.shape
    D = T * 128
    NB = S // R
    NSUB = R // SUB
    NCH = S // CH
    lqk, lv, lp = (lqk0, lqk1), (lv0, lv1), (lp0, lp1)
    step = pl.program_id(0)
    is_pre = step < NB
    blk = step % NB
    row0 = pl.multiple_of(blk * R, R)
    zero = jnp.minimum(step, 0)
    true = jnp.broadcast_to(zero, (8, 128)) == 0

    def x_copy(b, part=None):
        n = R if part is None else SUB
        rows = pl.ds(b * R + (part or 0) * SUB, n)
        sem = sems.at[b if part is None else part * NB]
        return pltpu.make_async_copy(x_hbm.at[rows], xin.at[rows], sem)

    def wq_copy(j):
        rows = pl.ds(j * 128, 128)
        return pltpu.make_async_copy(
            wq_hbm.at[rows], raw.at[rows, pl.ds(0, D)], sems.at[NB + 1 + j]
        )

    kv_copies = [
        pltpu.make_async_copy(src, wkv.at[i], sems.at[NB + 1 + T + i])
        for i, src in enumerate([wk_hbm, wv_hbm])
    ]

    def late_copy(i):
        src = [wqkv_hbm.at[:, pl.ds(p * D, D)] for p in range(3)] + [wob_hbm]
        return pltpu.make_async_copy(
            src[i], raw.at[:, pl.ds((i + 1) * D, D)], sems.at[NB + 3 + T + i]
        )

    woa_copies = [
        pltpu.make_async_copy(
            woa_hbm.at[:, _tile(t)], woa.at[pl.ds(t * D, D)], sems.at[NB + 7 + T + t]
        )
        for t in range(T)
    ]

    @pl.when(step == 0)
    def _():
        ahead = 3
        x_copy(0, 0).start()
        for j in range(ahead):
            wq_copy(j).start()
        for c in kv_copies:
            c.start()
        lqk1[:, SUB:, :] = jnp.zeros((2 * T, HALO, 128), F32)
        lv1[:, SUB:, :] = jnp.zeros((T, HALO, 128), F32)
        ot[...] = jnp.zeros(ot.shape, BF16)
        kmean[...] = jnp.zeros(kmean.shape, F32)
        x1[...] = jnp.zeros(x1.shape, F32)
        x_copy(0, 0).wait()

        def first_rows(j, _):
            pl.when(j + ahead < T)(wq_copy(jnp.minimum(j + ahead, T - 1)).start)
            pl.when(j + ahead == T)(x_copy(0, 1).start)
            wq_copy(j).wait()
            wt[j, 0:D // 2, :] = _pack(raw[_aligned(j, 128), 0:D].T)
            for g in range(SUB // T // LR):
                g = j * (SUB // T // LR) + g
                x = xin[_aligned(g, LR), :].astype(F32)
                ds, inv = _layernorm([x[:, _tile(t)] for t in range(T)])
                for t in range(T):
                    ln[t, _aligned(g, LR // 2), :] = _pack(ds[t] * inv)

        lax.fori_loop(0, T, first_rows, None)
        for i in (0, 3):
            late_copy(i).start()
        x_copy(1).start()
        for i, c in enumerate(kv_copies):
            c.wait()
            for j in range(T):
                wt[j, _half(slice(D + i * DH, D + (i + 1) * DH)), :] = _pack(wkv[i, :, _tile(j)])
        x_copy(0, 1).wait()

    for s, waits, starts in ((1, (0, 3), (1,)), (2, (1,), (2,)), (3, (2,), ())):
        @pl.when(step == s)
        def _():
            x_copy(s).wait()
            for i in waits:
                late_copy(i).wait()
            if s + 1 < NB:
                x_copy(s + 1).start()
            for i in starts:
                late_copy(i).start()
            if s == NB - 1:
                for c in woa_copies:
                    c.start()

    @pl.when(step == NB)
    def _():
        for c in woa_copies:
            c.wait()

    @pl.when(jnp.logical_and(is_pre, step > 0))
    def _():
        def first_rows(j, _):
            for g in range(64 // LR):
                g = j * (64 // LR) + g
                x = xin[_aligned(blk * (R // LR) + g, LR), :].astype(F32)
                ds, inv = _layernorm([x[:, _tile(t)] for t in range(T)])
                for t in range(T):
                    ln[t, _aligned(g, LR // 2), :] = _pack(ds[t] * inv)

        lax.fori_loop(0, SUB // 64, first_rows, None)

    @pl.when(step == 2 * NB)
    def _():
        for ref in (kb, kv, vt):
            n = ref.shape[1] // NB * (NB - 1)
            ref[0, 0:n] = ref[1, 0:n]

    @pl.when(step >= NB)
    def _():
        def load_q(h):
            return jnp.concatenate([_unpack(qt[blk, _aligned(h, DH // 2), :]), jnp.zeros((128 - DH, R), BF16)], axis=0)

        def spread_q(h, slot, unit, token):
            g, cols = unit // (R // 128), _tile(unit % (R // 128))
            w = qt[blk, _aligned(h * (DH // 16) + g, 8), cols]
            if token is not None:
                w = jnp.where(true, w, pltpu.bitcast(token, U32))
            for odd, y in enumerate((w << 16, w & np.uint32(0xFFFF0000))):
                y = pltpu.bitcast(y, F32)
                for i in range(8):
                    qb[slot, 16 * g + 2 * i + odd, :, cols] = jnp.broadcast_to(y[i:i + 1], (8, 128))

        def scores(q, c):
            return _dot(_unpack(kb[0, _half(slice(c * CH, c * CH + MK)), :]), q)

        def tokens(s, pv):
            return [y[r:r + 8, 0:128] for y in (s, pv) if y is not None for r in range(0, len(y), 8)]

        def probs(s, slot, c, tok):
            acc = None
            for d in range(DH):
                token = jnp.concatenate([tok[d * len(tok) // DH]] * (VK // 8), axis=0)
                k = kv[0, c, d]
                if d % GS == 0:
                    k = jnp.where(jnp.concatenate([true] * (VK // 8), axis=0), k, token)
                y = _lanes([k] * (R // 128)) * jnp.concatenate([qb[slot, d]] * (VK // 8), axis=0)
                acc = y if acc is None else acc + y
            p = jnp.exp2(jnp.concatenate([s, acc], axis=0))
            return p.astype(BF16), p.reshape(CH // 8, 8, R).sum(axis=0)

        def fast_heads(it, carry):
            low, every = carry
            heads = [jnp.minimum(it * HU + u, H - 1) for u in range(HU + 1)]
            qs = [load_q(h) for h in heads]
            p, l = _unpack(p0[...]), l0[...]
            for u in range(HU):
                acc = None
                for c in range(NCH):
                    v, c2 = (u + (c + 1) // NCH), (c + 1) % NCH
                    s = scores(qs[v], c2)
                    n = CH // 128
                    pv = _dot(_lanes([_unpack(vt[0, c * n + j]) for j in range(n)]), p)
                    acc = pv if acc is None else acc + pv
                    tok = tokens(s, pv)
                    p, l_next = probs(s, v % HU, c2, tok)
                    if c2:
                        l = l + l_next
                        units = range(c * UNITS // (NCH - 1), c2 * UNITS // (NCH - 1))
                        for i, unit in enumerate(units):
                            spread_q(heads[u + 1], (u + 1) % HU, unit, tok[-1 - 15 * i])
                    if u == 0 and c == 2:
                        token = pltpu.bitcast(jnp.concatenate([s[:8, 0:128]] * 8, axis=0), U32)
                        w = pltpu.bitcast(ot[...], U32)
                        mask = jnp.concatenate([true] * 8, axis=0)
                        w = _lanes([jnp.where(mask, w[:, _tile(j)], token) for j in range(R // 128)])
                        oa[(it + T - 1) % T] = _pack(_unpack(w).T)
                total = jnp.sum(l, axis=0, keepdims=True)
                l = l_next
                ot[u * DH:(u + 1) * DH, :] = (acc * (1.0 / total)).astype(BF16)
                low = jnp.minimum(low, total)
                every = every + acc.reshape(DH // 8, 8, R).sum(axis=0) + total
            p0[...] = pltpu.bitcast(p, U32)
            l0[...] = l
            return low, every

        for unit in range(UNITS):
            spread_q(0, 0, unit, None)
        s = scores(load_q(0), 0)
        p, l = probs(s, 0, 0, [s[:8, 0:128]])
        p0[...] = pltpu.bitcast(p, U32)
        l0[...] = l
        low, every = lax.fori_loop(
            0, H // HU, fast_heads, (jnp.ones((1, R), F32), jnp.zeros((8, R), F32))
        )
        ok = jnp.where(jnp.logical_and(low >= 1.0, jnp.abs(every) < 3e38), 1.0, 0.0)

        @pl.when(zero == 0)
        def _():
            oa[T - 1] = _pack(ot[...].T)

        @pl.when(jnp.min(ok) < 1.0)
        def _():
            def safe_tile(tile, _):
                def safe_head(u, _):
                    q = load_q(tile * HU + u)

                    def chunk(c, carry):
                        m, l, acc = carry
                        s = _dot(_unpack(kb[0, _aligned(c, 64), :]), q)
                        m_new = jnp.maximum(m, jnp.max(s, axis=0, keepdims=True))
                        alpha = jnp.exp2(m - m_new)
                        p = jnp.exp2(s - m_new)
                        l = alpha * l + jnp.sum(p, axis=0, keepdims=True)
                        acc = alpha * acc + _dot(_unpack(vt[0, c]), p.astype(BF16))
                        return m_new, l, acc

                    init = (
                        jnp.full((1, R), -jnp.inf, F32),
                        jnp.zeros((1, R), F32),
                        jnp.zeros((DH, R), F32),
                    )
                    _, l, acc = lax.fori_loop(0, S // 128, chunk, init)
                    ot[_aligned(u, DH), :] = (acc / l).astype(BF16)

                lax.fori_loop(0, HU, safe_head, None)
                oa[tile] = _pack(ot[...].T)

            lax.fori_loop(0, T, safe_tile, None)

        first = blk == 0

        def sub(i):
            return slice(i * SUB, (i + 1) * SUB)

        def gated(c, token):
            return jnp.where(true, c, token)

        def operand(ref, i):
            return _lanes([_unpack(ref[k, _half(sub(i)), :]) for k in range(T)])

        def packed(ref, i):
            held = []

            def store(r, ys, scale):
                if not held:
                    return held.append((ys, scale))
                before, scale0 = held.pop()
                scale = jnp.concatenate([scale0, scale], axis=0)
                for t, pair in enumerate(zip(before, ys)):
                    pair = jnp.concatenate(pair, axis=0) * scale
                    ref[t, (i * SUB + r - 8) // 2:(i * SUB + r + 8) // 2, :] = _pack(pair)

            return store

        def out_proj_a(i):
            def piece(t):
                y = _dot(operand(oa, i), woa[t * D:(t + 1) * D, :])
                y = y + xs[t, _aligned(blk * NSUB + i, SUB), :]
                x1[t, sub(i), :] = y
                return _in_time_order(y)

            return [functools.partial(piece, t) for t in range(T)]

        def norm(i):
            store = packed(ln, i)

            def piece(r, token):
                x = [x1[t, i * SUB + r:i * SUB + r + 8, :] for t in range(T)]
                x[0] = gated(x[0], token)
                store(r, *_layernorm(x))

            return [functools.partial(piece, r) for r in range(0, SUB, 8)]

        def qkv_proj(i, part):
            def piece(t):
                z = _dot(operand(ln, i), _unpack(wqkv[(part + 1) * T + t]))
                if part == 0:
                    lqk[i][t, HALO:, :] = z
                    return _in_time_order(z)
                refs, t = (lqk, T + t) if part == 1 else (lv, t)
                if i == 0:
                    refs[0][t, 0:HALO, :] = jnp.where(first, z[0:1, :], refs[-1][t, SUB:, :])
                if i + 1 < NSUB:
                    refs[i + 1][t, 0:HALO, :] = z[SUB - HALO:, :]
                refs[i][t, HALO:, :] = z
                return _in_time_order(z)

            return [functools.partial(piece, t) for t in range(T)]

        def window(r, w):
            return slice(HALO + r - DIL * w, HALO + r - DIL * w + 8)

        def local_probs(i):
            def piece(r, token):
                scale = gated(QSCALE, token)
                q = [lqk[i][t, window(r, 0), :] * scale for t in range(T)]
                z = []
                for w in range(W):
                    y = functools.reduce(jnp.add, [
                        q[t] * lqk[i][T + t, window(r, w), :] for t in range(T)
                    ])
                    y = y + pltpu.roll(y, 64, 1)
                    y = y + pltpu.roll(y, 32, 1)
                    if i == 0 and r < DIL * w:
                        pos = row0 + r + lax.broadcasted_iota(jnp.int32, (8, 128), 0)
                        y = jnp.where(pos >= DIL * w, y, MASKED)
                    z.append(y)
                m = functools.reduce(jnp.maximum, z)
                e = [jnp.exp2(y - m) for y in z]
                for w in range(W):
                    lp[i][w, r:r + 8, :] = e[w]
                lp[i][W, r:r + 8, :] = 1.0 / functools.reduce(jnp.add, e)

            return [functools.partial(piece, r) for r in range(0, SUB, 8)]

        def local_values(i):
            store = packed(ob, i)

            def piece(r, token):
                p = [gated(lp[i][w, r:r + 8, :], token) for w in range(W)]
                store(r, [
                    functools.reduce(jnp.add, [p[w] * lv[i][t, window(r, w), :] for w in range(W)])
                    for t in range(T)
                ], lp[i][W, r:r + 8, :])

            return [functools.partial(piece, r) for r in range(0, SUB, 8)]

        def out_proj_b(i):
            def piece(t):
                y = _dot(operand(ob, i), _unpack(wob[T + t]))
                y = y + x1[t, sub(i), :]
                x1[t, sub(i), :] = y
                o_ref[sub(i), _tile(t)] = y.astype(BF16)
                return _in_time_order(y)

            return [functools.partial(piece, t) for t in range(T)]

        def run(mxu, vpu):
            _interleave(mxu, (vpu, 0, len(mxu) - 1))

        Q, K, V = range(3)
        _interleave(out_proj_a(0))
        run(out_proj_a(1), norm(0))
        run(qkv_proj(0, K) + qkv_proj(0, Q), norm(1))
        run(qkv_proj(1, K) + qkv_proj(1, Q), local_probs(0))
        run(qkv_proj(0, V), local_probs(1))
        run(qkv_proj(1, V), local_values(0))
        run(out_proj_b(0), local_values(1))
        run(out_proj_b(1), norm(0))

    @pl.when(step < 2 * NB)
    def _():
        slot = jnp.where(jnp.logical_and(step >= NB, blk < NB - 1), 1, 0)
        part = jnp.where(is_pre, step, 0)

        def gated(x, token):
            token = pltpu.bitcast(token, x.dtype)
            return jnp.concatenate(
                [jnp.where(true, x[r:r + 8], token) for r in range(0, x.shape[0], 8)], axis=0
            )

        def cols_in(c, g, token):
            w = pltpu.bitcast(raw[c * 256:(c + 1) * 256, _aligned(part * T + g, 128)], U32)
            w = gated(w, token).T
            for u in range(4):
                tmp_c[c % 2, pl.ds((4 * g + u) * PAD, DH), :] = w[u * DH:(u + 1) * DH]

        def cols_out(c, g, token):
            w = jnp.concatenate(
                [tmp_c[c % 2, pl.ds(4 * g + u, H, stride=PAD), :] for u in range(4)], axis=0
            )
            wqkv[part * T + g, _tile(c), :] = gated(w, token).T

        def wob_tile(i):
            j = jnp.where(part > 0, jnp.minimum(T + 3 * (part - 1) + i, 2 * T - 1), i)
            return j, jnp.where(part > 0, 3 * T + j, j)

        def rows_in(i, n, token):
            w = raw[n * 2 * DH:(n + 1) * 2 * DH, _aligned(wob_tile(i)[1], 128)]
            tmp_r[pl.ds(n * PAD, DH), :] = gated(pltpu.bitcast(w, U32), token)

        def rows_out(i, e, token):
            token = pltpu.bitcast(jnp.concatenate([token] * 2, axis=0), U32)
            low = jnp.where(jnp.concatenate([true] * 2, axis=0), np.uint32(0xFFFF), token)
            a = tmp_r[pl.ds(e, H // 2, stride=PAD), :]
            b = tmp_r[pl.ds(DH // 2 + e, H // 2, stride=PAD), :]
            even = (a & low) | (b << 16)
            odd = (a >> 16) | (b & ~low)
            wob[wob_tile(i)[0], e * H:(e + 1) * H, :] = jnp.concatenate([even, odd], axis=0)

        def place_rows(r, token):
            rows = _aligned(blk * (R // LR) + r // LR, LR)
            x = xin[rows, :].astype(F32)
            mask = jnp.concatenate([jnp.logical_and(true, is_pre)] * (LR // 8), axis=0)
            x = [
                jnp.where(mask, x[:, _tile(t)], gated(x1[t, r:r + LR, :], token)) for t in range(T)
            ]
            for t in range(T):
                xs[t, rows, :] = x[t]
            if r >= SUB:
                ds, inv = _layernorm(x)
                for t in range(T):
                    ln[t, r // 2:(r + LR) // 2, :] = _pack(ds[t] * inv)

        NM = 4
        MR = (D + 2 * DH) // NM

        def project(j, m):
            z = lax.dot_general(
                _lanes([_unpack(wt[t, m * MR // 2:(m + 1) * MR // 2, :]) for t in range(T)]),
                _lanes([_unpack(ln[t, _half(_tile(j)), :]) for t in range(T)]),
                NT, preferred_element_type=F32,
            )
            nq = min(MR, D - m * MR)
            qt[blk, m * MR // 2:(m * MR + nq) // 2, _tile(j)] = _pack(z[:nq])
            if nq == MR:
                return _in_time_order(z)
            n = blk * (R // 128) + j
            vt[slot, n] = _pack(z[nq + DH:])
            k = z[nq:nq + DH]
            if j == 0:
                mean = jnp.sum(k, axis=-1, keepdims=True) * (1.0 / 128)
                kmean[...] = jnp.where(jnp.broadcast_to(blk, (DH, 128)) == 0, mean, kmean[...])
            k = ((k - kmean[...]) * QSCALE).astype(BF16).astype(F32)
            k = jnp.concatenate([k, jnp.zeros((128 - DH, 128), F32)], axis=0).T
            kb[slot, _aligned(n, 64), :] = _pack(k)
            if j % (CH // 128) == CH // 128 - 1:
                for d in range(DH):
                    kv[slot, n // (CH // 128), d] = jnp.broadcast_to(
                        k[128 - VK:, d:d + 1], (VK, 128)
                    )
            return _in_time_order(z)

        part_ = functools.partial
        nc = D // 256
        order = [(cols_in, 0)]
        for c in range(nc):
            order += [(cols_in, c + 1)] * (c + 1 < nc) + [(cols_out, c)]
        end = NM * R // 128
        _interleave(
            [part_(project, j, m) for j in range(R // 128) for m in reversed(range(NM))],
            ([part_(place_rows, r) for r in range(SUB, R, LR)], 0, end // 2 - 2),
            ([part_(place_rows, r) for r in range(0, SUB, LR)], end // 2, end - 1),
            ([part_(f, c, g) for f, c in order for g in range(T)], 0, end - 1),
            ([part_(f, i, n) for i in range(3) for f in (rows_in, rows_out) for n in range(16)],
             0, end - 1),
        )


@jax.jit
def pallas_interleave_layers__grouped_kv_mqa__sliding_local_dilated__prompt_kernel(
    A_x: jax.Array,
    A_wq: jax.Array,
    A_wk: jax.Array,
    A_wv: jax.Array,
    A_wo: jax.Array,
    B_x: jax.Array,
    B_wqkv: jax.Array,
    B_wo: jax.Array,
):
    del B_x
    _, S, D = A_x.shape
    NB = S // R
    T = D // 128
    vmem = pltpu.VMEM
    out = pl.pallas_call(
        _kernel,
        grid=(3 * NB,),
        in_specs=[pl.BlockSpec(memory_space=pl.ANY)] * 7,
        out_specs=pl.BlockSpec((R, D), lambda s: (jnp.maximum(s - 2 * NB, 0), 0)),
        out_shape=jax.ShapeDtypeStruct((S, D), A_x.dtype),
        scratch_shapes=[
            vmem((S, D), BF16),
            vmem((D, 5 * D), BF16),
            vmem((2, DH, D), BF16),
            vmem((T, D // 2 + DH, 128), U32),
            vmem((T * D, 128), BF16),
            vmem((4 * T, D // 2, 128), U32),
            vmem((2 * T, D // 2, 128), U32),
            vmem((2, H * PAD, 128), U32),
            vmem((H // 2 * PAD, 128), U32),
            vmem((T, S, 128), F32),
            vmem((T, R, 128), F32),
            vmem((T, R // 2, 128), U32),
            vmem((NB, D // 2, R), U32),
            vmem((DH, 128), F32),
            vmem((2, S // 2, 128), U32),
            vmem((2, S // CH, DH, VK, 128), F32),
            vmem((2, S // 128, DH // 2, 128), U32),
            vmem((HU, DH, 8, R), F32),
            vmem((CH // 2, R), U32),
            vmem((8, R), F32),
            vmem((128, R), BF16),
            vmem((T, R // 2, 128), U32),
            vmem((T, R // 2, 128), U32),
            vmem((2 * T, HALO + SUB, 128), F32),
            vmem((2 * T, HALO + SUB, 128), F32),
            vmem((T, HALO + SUB, 128), F32),
            vmem((T, HALO + SUB, 128), F32),
            vmem((W + 1, SUB, 128), F32),
            vmem((W + 1, SUB, 128), F32),
            pltpu.SemaphoreType.DMA((NB + 2 * T + 7,)),
        ],
        compiler_params=pltpu.CompilerParams(
            dimension_semantics=("arbitrary",),
            vmem_limit_bytes=110 * 2**20,
        ),
        name="interleave_layers",
    )(A_x.reshape(S, D), A_wq, A_wk.T, A_wv.T, A_wo, B_wqkv, B_wo)
    return out.reshape(1, S, D)
```

```python
import functools
import math

import jax
import jax.numpy as jnp
import numpy as np
from jax import lax
from jax.experimental import pallas as pl
from jax.experimental.pallas import tpu as pltpu

F32 = jnp.float32
BF16 = jnp.bfloat16
U32 = jnp.uint32

H = 32
DH = 32
W = 8
DIL = 2
HALO = 16
EPS = 1e-5
QSCALE = DH ** -0.5 * math.log2(math.e)
MASKED = -1e9 * math.log2(math.e)

R = 512
SUB = 256
CH = 256
VK = 16
MK = CH - VK
GS = 2
HU = 4
UNITS = DH // 16 * R // 128
LR = 16
PAD = 33

NT = (((1,), (1,)), ((), ()))


def _layernorm(xs):
    inv_d = 1.0 / (128 * len(xs))
    m = jnp.sum(functools.reduce(jnp.add, xs), axis=-1, keepdims=True) * inv_d
    ds = [x - m for x in xs]
    v = jnp.sum(functools.reduce(jnp.add, [d * d for d in ds]), axis=-1, keepdims=True) * inv_d
    return ds, lax.rsqrt(v + EPS)


def _pack(x):
    return pltpu.bitcast(x.astype(BF16), U32)


def _unpack(x):
    return pltpu.bitcast(x, BF16)


def _half(rows):
    return slice(rows.start // 2, rows.stop // 2)


def _aligned(index, n):
    return pl.ds(pl.multiple_of(index * n, n), n)


def _dot(a, b):
    return jnp.dot(a, b, preferred_element_type=F32)


def _lanes(tiles):
    return jnp.concatenate(tiles, axis=1)


def _tile(t):
    return slice(t * 128, (t + 1) * 128)


def _in_time_order(y):
    return [y[r:r + 8, 0:128] for r in range(0, y.shape[0], 8)]


def _interleave(mxu, *jobs):
    todo = sorted(
        [(start + (stop - start) * i / len(pieces), j, i, piece)
         for j, (pieces, start, stop) in enumerate(jobs) for i, piece in enumerate(pieces)],
        key=lambda item: item[:3],
    )
    for n, piece in enumerate(mxu):
        results = piece()
        while todo and todo[0][0] < n + 1:
            at, _, _, other = todo.pop(0)
            other(results[int((at - n) * len(results))])
    assert not todo


def _kernel(
    x_hbm, wq_hbm, wk_hbm, wv_hbm, woa_hbm, wqkv_hbm, wob_hbm,
    o_ref,
    xin, raw, wkv, wt, woa, wqkv, wob, tmp_c, tmp_r,
    xs, x1, ln, qt, kmean, kb, kv, vt, qb, p0, l0, ot, oa, ob,
    lqk0, lqk1, lv0, lv1, lp0, lp1,
    sems,
):
    T, S, _ = xs.shape
    D = T * 128
    NB = S // R
    NSUB = R // SUB
    NCH = S // CH
    lqk, lv, lp = (lqk0, lqk1), (lv0, lv1), (lp0, lp1)
    step = pl.program_id(0)
    is_pre = step < NB
    blk = step % NB
    row0 = pl.multiple_of(blk * R, R)
    zero = jnp.minimum(step, 0)
    true = jnp.broadcast_to(zero, (8, 128)) == 0

    NX = S // SUB

    def x_copy(i):
        rows = pl.ds(i * SUB, SUB)
        return pltpu.make_async_copy(x_hbm.at[rows], xin.at[rows], sems.at[i])

    def wq_copy(j):
        rows = pl.ds(j * 128, 128)
        return pltpu.make_async_copy(
            wq_hbm.at[rows], raw.at[rows, pl.ds(0, D)], sems.at[NX + j]
        )

    kv_copies = [
        pltpu.make_async_copy(src, wkv.at[i], sems.at[NX + T + i])
        for i, src in enumerate([wk_hbm, wv_hbm])
    ]

    def late_copy(i):
        src = [wqkv_hbm.at[:, pl.ds(p * D, D)] for p in range(3)] + [wob_hbm]
        return pltpu.make_async_copy(
            src[i], raw.at[:, pl.ds((i + 1) * D, D)], sems.at[NX + 2 + T + i]
        )

    woa_copies = [
        pltpu.make_async_copy(
            woa_hbm.at[:, _tile(t)], woa.at[pl.ds(t * D, D)], sems.at[NX + 6 + T + t]
        )
        for t in range(T)
    ]

    @pl.when(step == 0)
    def _():
        ahead = 4
        x_copy(0).start()
        for j in range(ahead):
            wq_copy(j).start()
        for c in kv_copies:
            c.start()
        lqk1[:, SUB:, :] = jnp.zeros((2 * T, HALO, 128), F32)
        lv1[:, SUB:, :] = jnp.zeros((T, HALO, 128), F32)
        ot[...] = jnp.zeros(ot.shape, BF16)
        kmean[...] = jnp.zeros(kmean.shape, F32)
        x1[...] = jnp.zeros(x1.shape, F32)
        x_copy(0).wait()

        n = 2

        def first_rows(i, _):
            for u in range(n):
                j = i * n + u
                pl.when(j + ahead < T)(wq_copy(jnp.minimum(j + ahead, T - 1)).start)
                pl.when(j + ahead == T)(x_copy(1).start)
                pl.when(j + ahead == T + 1)(x_copy(2).start)
                wq_copy(j).wait()
            for u in range(n):
                j = i * n + u
                wt[j, 0:D // 2, :] = _pack(raw[_aligned(j, 128), 0:D].T)
                for g in range(SUB // T // LR):
                    g = j * (SUB // T // LR) + g
                    x = xin[_aligned(g, LR), :].astype(F32)
                    ds, inv = _layernorm([x[:, _tile(t)] for t in range(T)])
                    for t in range(T):
                        ln[t, _aligned(g, LR // 2), :] = _pack(ds[t] * inv)

        lax.fori_loop(0, T // n, first_rows, None)
        for i, c in enumerate(kv_copies):
            c.wait()
            for j in range(T):
                wt[j, _half(slice(D + i * DH, D + (i + 1) * DH)), :] = _pack(wkv[i, :, _tile(j)])

    for s, waits, starts in ((0, (), (0, 3)), (1, (0, 3), (1,)), (2, (1,), (2,)), (3, (2,), ())):
        @pl.when(step == s)
        def _():
            for i in range(NSUB * s + 1, min(NSUB * (s + 1) + 1, NX)):
                x_copy(i).wait()
            for i in waits:
                late_copy(i).wait()
            for i in range(NSUB * (s + 1) + 1, min(NSUB * (s + 2) + 1, NX)):
                x_copy(i).start()
            for i in starts:
                late_copy(i).start()
            if s == NB - 1:
                for c in woa_copies:
                    c.start()

    @pl.when(step == NB)
    def _():
        for c in woa_copies:
            c.wait()

    @pl.when(step == 2 * NB)
    def _():
        for ref in (kb, kv, vt):
            n = ref.shape[1] // NB * (NB - 1)
            ref[0, 0:n] = ref[1, 0:n]

    @pl.when(step >= NB)
    def _():
        def load_q(h):
            return jnp.concatenate([_unpack(qt[_aligned(jnp.minimum(blk * H + h, NB * H - 1), DH // 2), :]), jnp.zeros((128 - DH, R), BF16)], axis=0)

        def spread_q(h, slot, unit, token):
            g, cols = unit // (R // 128), _tile(unit % (R // 128))
            w = qt[_aligned(jnp.minimum(blk * H + h, NB * H - 1) * (DH // 16) + g, 8), cols]
            if token is not None:
                w = jnp.where(true, w, pltpu.bitcast(token, U32))
            for odd, y in enumerate((w << 16, w & np.uint32(0xFFFF0000))):
                y = pltpu.bitcast(y, F32)
                for i in range(8):
                    qb[slot, 16 * g + 2 * i + odd, :, cols] = jnp.broadcast_to(y[i:i + 1], (8, 128))

        def scores(q, c):
            return _dot(_unpack(kb[0, _half(slice(c * CH, c * CH + MK)), :]), q)

        def tokens(s, pv):
            return [y[r:r + 8, 0:128] for y in (s, pv) if y is not None for r in range(0, len(y), 8)]

        def probs(s, slot, c, tok):
            acc = None
            for d in range(DH):
                token = jnp.concatenate([tok[d * len(tok) // DH]] * (VK // 8), axis=0)
                k = kv[0, c, d]
                if d % GS == 0:
                    k = jnp.where(jnp.concatenate([true] * (VK // 8), axis=0), k, token)
                y = _lanes([k] * (R // 128)) * jnp.concatenate([qb[slot, d]] * (VK // 8), axis=0)
                acc = y if acc is None else acc + y
            p = jnp.exp2(jnp.concatenate([s, acc], axis=0))
            return p.astype(BF16), p.reshape(CH // 8, 8, R).sum(axis=0)

        def fast_heads(it, carry):
            low, every = carry
            heads = [it * HU + u for u in range(HU + 1)]
            qs = [load_q(h) for h in heads]
            p, l = _unpack(p0[...]), l0[...]
            for u in range(HU):
                acc = None
                for c in range(NCH):
                    v, c2 = (u + (c + 1) // NCH), (c + 1) % NCH
                    s = scores(qs[v], c2)
                    n = CH // 128
                    pv = _dot(_lanes([_unpack(vt[0, c * n + j]) for j in range(n)]), p)
                    acc = pv if acc is None else acc + pv
                    tok = tokens(s, pv)
                    p, l_next = probs(s, v % HU, c2, tok)
                    if c2:
                        l = l + l_next
                        units = range(c * UNITS // (NCH - 1), c2 * UNITS // (NCH - 1))
                        for i, unit in enumerate(units):
                            spread_q(heads[u + 1], (u + 1) % HU, unit, tok[-1 - 15 * i])
                    if u == 0 and c == 2:
                        token = pltpu.bitcast(jnp.concatenate([s[:8, 0:128]] * 8, axis=0), U32)
                        w = pltpu.bitcast(ot[...], U32)
                        mask = jnp.concatenate([true] * 8, axis=0)
                        w = _lanes([jnp.where(mask, w[:, _tile(j)], token) for j in range(R // 128)])
                        oa[(it + T - 1) % T] = _pack(_unpack(w).T)
                total = jnp.sum(l, axis=0, keepdims=True)
                l = l_next
                ot[u * DH:(u + 1) * DH, :] = (acc * (1.0 / total)).astype(BF16)
                low = jnp.minimum(low, total)
                every = every + acc.reshape(DH // 8, 8, R).sum(axis=0) + total
            p0[...] = pltpu.bitcast(p, U32)
            l0[...] = l
            return low, every

        @pl.when(blk == 0)
        def _():
            for unit in range(UNITS):
                spread_q(0, 0, unit, None)
            s = scores(load_q(0), 0)
            p, l = probs(s, 0, 0, [s[:8, 0:128]])
            p0[...] = pltpu.bitcast(p, U32)
            l0[...] = l

        low, every = lax.fori_loop(
            0, H // HU, fast_heads, (jnp.ones((1, R), F32), jnp.zeros((8, R), F32))
        )

        def fallback():
            def safe_tile(tile, _):
                def safe_head(u, _):
                    q = load_q(tile * HU + u)

                    def chunk(c, carry):
                        m, l, acc = carry
                        s = _dot(_unpack(kb[0, _aligned(c, 64), :]), q)
                        m_new = jnp.maximum(m, jnp.max(s, axis=0, keepdims=True))
                        alpha = jnp.exp2(m - m_new)
                        p = jnp.exp2(s - m_new)
                        l = alpha * l + jnp.sum(p, axis=0, keepdims=True)
                        acc = alpha * acc + _dot(_unpack(vt[0, c]), p.astype(BF16))
                        return m_new, l, acc

                    init = (
                        jnp.full((1, R), -jnp.inf, F32),
                        jnp.zeros((1, R), F32),
                        jnp.zeros((DH, R), F32),
                    )
                    _, l, acc = lax.fori_loop(0, S // 128, chunk, init)
                    ot[_aligned(u, DH), :] = (acc / l).astype(BF16)

                lax.fori_loop(0, HU, safe_head, None)
                oa[tile] = _pack(ot[...].T)

            lax.fori_loop(0, T, safe_tile, None)

        @pl.when(zero == 0)
        def _():
            oa[T - 1] = _pack(ot[...].T)
            ok = jnp.where(jnp.logical_and(low >= 1.0, jnp.abs(every) < 3e38), 1.0, 0.0)
            pl.when(jnp.min(ok) < 1.0)(fallback)

        first = blk == 0

        def sub(i):
            return slice(i * SUB, (i + 1) * SUB)

        def gated(c, token):
            return jnp.where(true, c, token)

        def operand(ref, i):
            return _lanes([_unpack(ref[k, _half(sub(i)), :]) for k in range(T)])

        def packed(ref, i):
            held = []

            def store(r, ys, scale):
                if not held:
                    return held.append((ys, scale))
                before, scale0 = held.pop()
                scale = jnp.concatenate([scale0, scale], axis=0)
                for t, pair in enumerate(zip(before, ys)):
                    pair = jnp.concatenate(pair, axis=0) * scale
                    ref[t, (i * SUB + r - 8) // 2:(i * SUB + r + 8) // 2, :] = _pack(pair)

            return store

        def out_proj_a(i):
            def piece(t):
                y = _dot(operand(oa, i), woa[t * D:(t + 1) * D, :])
                y = y + xs[t, _aligned(blk * NSUB + i, SUB), :]
                x1[t, sub(i), :] = y
                return _in_time_order(y)

            return [functools.partial(piece, t) for t in range(T)]

        def norm(i):
            store = packed(ln, i)

            def piece(r, token):
                x = [x1[t, i * SUB + r:i * SUB + r + 8, :] for t in range(T)]
                x[0] = gated(x[0], token)
                store(r, *_layernorm(x))

            return [functools.partial(piece, r) for r in range(0, SUB, 8)]

        def qkv_proj(i, part):
            def piece(t):
                z = _dot(operand(ln, i), _unpack(wqkv[(part + 1) * T + t]))
                if part == 0:
                    lqk[i][t, HALO:, :] = z
                    return _in_time_order(z)
                refs, t = (lqk, T + t) if part == 1 else (lv, t)
                if i == 0:
                    refs[0][t, 0:HALO, :] = jnp.where(first, z[0:1, :], refs[-1][t, SUB:, :])
                if i + 1 < NSUB:
                    refs[i + 1][t, 0:HALO, :] = z[SUB - HALO:, :]
                refs[i][t, HALO:, :] = z
                return _in_time_order(z)

            return [functools.partial(piece, t) for t in range(T)]

        def window(r, w):
            return slice(HALO + r - DIL * w, HALO + r - DIL * w + 8)

        def local_probs(i):
            def piece(r, token):
                scale = gated(QSCALE, token)
                q = [lqk[i][t, window(r, 0), :] * scale for t in range(T)]
                z = []
                for w in range(W):
                    y = functools.reduce(jnp.add, [
                        q[t] * lqk[i][T + t, window(r, w), :] for t in range(T)
                    ])
                    y = y + pltpu.roll(y, 64, 1)
                    y = y + pltpu.roll(y, 32, 1)
                    if i == 0 and r < DIL * w:
                        pos = row0 + r + lax.broadcasted_iota(jnp.int32, (8, 128), 0)
                        y = jnp.where(pos >= DIL * w, y, MASKED)
                    z.append(y)
                m = functools.reduce(jnp.maximum, z)
                e = [jnp.exp2(y - m) for y in z]
                for w in range(W):
                    lp[i][w, r:r + 8, :] = e[w]
                lp[i][W, r:r + 8, :] = 1.0 / functools.reduce(jnp.add, e)

            return [functools.partial(piece, r) for r in range(0, SUB, 8)]

        def local_values(i):
            store = packed(ob, i)

            def piece(r, token):
                p = [gated(lp[i][w, r:r + 8, :], token) for w in range(W)]
                store(r, [
                    functools.reduce(jnp.add, [p[w] * lv[i][t, window(r, w), :] for w in range(W)])
                    for t in range(T)
                ], lp[i][W, r:r + 8, :])

            return [functools.partial(piece, r) for r in range(0, SUB, 8)]

        def out_proj_b(i):
            def piece(t):
                y = _dot(operand(ob, i), _unpack(wob[T + t]))
                y = y + x1[t, sub(i), :]
                x1[t, sub(i), :] = y
                o_ref[sub(i), _tile(t)] = y.astype(BF16)
                return _in_time_order(y)

            return [functools.partial(piece, t) for t in range(T)]

        def run(mxu, vpu):
            _interleave(mxu, (vpu, 0, len(mxu) - 1))

        Q, K, V = range(3)
        _interleave(out_proj_a(0))
        run(out_proj_a(1), norm(0))
        run(qkv_proj(0, K) + qkv_proj(0, Q), norm(1))
        run(qkv_proj(1, K) + qkv_proj(1, Q), local_probs(0))
        run(qkv_proj(0, V), local_probs(1))
        run(qkv_proj(1, V), local_values(0))
        run(out_proj_b(0), local_values(1))
        run(out_proj_b(1), norm(0))

    @pl.when(step < 2 * NB)
    def _():
        slot = jnp.where(jnp.logical_and(step >= NB, blk < NB - 1), 1, 0)
        part = jnp.where(is_pre, step, 0)

        def gated(x, token):
            token = pltpu.bitcast(token, x.dtype)
            return jnp.concatenate(
                [jnp.where(true, x[r:r + 8], token) for r in range(0, x.shape[0], 8)], axis=0
            )

        def cols_in(c, g, token):
            w = pltpu.bitcast(raw[c * 256:(c + 1) * 256, _aligned(part * T + g, 128)], U32)
            w = gated(w, token).T
            for u in range(4):
                tmp_c[c % 2, pl.ds((4 * g + u) * PAD, DH), :] = w[u * DH:(u + 1) * DH]

        def cols_out(c, g, token):
            w = jnp.concatenate(
                [tmp_c[c % 2, pl.ds(4 * g + u, H, stride=PAD), :] for u in range(4)], axis=0
            )
            wqkv[part * T + g, _tile(c), :] = gated(w, token).T

        def wob_tile(i):
            j = jnp.where(part > 0, jnp.minimum(T + 3 * (part - 1) + i, 2 * T - 1), i)
            return j, jnp.where(part > 0, 3 * T + j, j)

        def rows_in(i, n, token):
            w = raw[n * 2 * DH:(n + 1) * 2 * DH, _aligned(wob_tile(i)[1], 128)]
            tmp_r[pl.ds(n * PAD, DH), :] = gated(pltpu.bitcast(w, U32), token)

        def rows_out(i, e, token):
            token = pltpu.bitcast(jnp.concatenate([token] * 2, axis=0), U32)
            low = jnp.where(jnp.concatenate([true] * 2, axis=0), np.uint32(0xFFFF), token)
            a = tmp_r[pl.ds(e, H // 2, stride=PAD), :]
            b = tmp_r[pl.ds(DH // 2 + e, H // 2, stride=PAD), :]
            even = (a & low) | (b << 16)
            odd = (a >> 16) | (b & ~low)
            wob[wob_tile(i)[0], e * H:(e + 1) * H, :] = jnp.concatenate([even, odd], axis=0)

        following = (blk + 1) % NB

        def load_x(b, r):
            x = xin[_aligned(b * (R // LR) + r // LR, LR), :].astype(F32)
            return [x[:, _tile(t)] for t in range(T)]

        def norm_rows(x, r):
            ds, inv = _layernorm(x)
            for t in range(T):
                ln[t, r // 2:(r + LR) // 2, :] = _pack(ds[t] * inv)

        def place_rows(r, token):
            mask = jnp.concatenate([jnp.logical_and(true, is_pre)] * (LR // 8), axis=0)
            x = [
                jnp.where(mask, y, gated(x1[t, r:r + LR, :], token))
                for t, y in enumerate(load_x(blk, r))
            ]
            for t in range(T):
                xs[t, _aligned(blk * (R // LR) + r // LR, LR), :] = x[t]
            if r >= SUB:
                norm_rows(x, r)
                return
            norm_rows([gated(y, token) for y in load_x(following, r)], r)

        NM = 4
        MR = (D + 2 * DH) // NM

        def project(j, m):
            z = lax.dot_general(
                _lanes([_unpack(wt[t, m * MR // 2:(m + 1) * MR // 2, :]) for t in range(T)]),
                _lanes([_unpack(ln[t, _half(_tile(j)), :]) for t in range(T)]),
                NT, preferred_element_type=F32,
            )
            nq = min(MR, D - m * MR)
            qt[pl.ds(pl.multiple_of(blk * (D // 2) + m * MR // 2, 8), nq // 2), _tile(j)] = _pack(z[:nq])
            if nq == MR:
                return _in_time_order(z)
            n = blk * (R // 128) + j
            vt[slot, n] = _pack(z[nq + DH:])
            k = z[nq:nq + DH]
            if j == 0:
                mean = jnp.sum(k, axis=-1, keepdims=True) * (1.0 / 128)
                kmean[...] = jnp.where(jnp.broadcast_to(blk, (DH, 128)) == 0, mean, kmean[...])
            k = ((k - kmean[...]) * QSCALE).astype(BF16).astype(F32)
            k = jnp.concatenate([k, jnp.zeros((128 - DH, 128), F32)], axis=0).T
            kb[slot, _aligned(n, 64), :] = _pack(k)
            if j % (CH // 128) == CH // 128 - 1:
                for d in range(DH):
                    kv[slot, n // (CH // 128), d] = jnp.broadcast_to(
                        k[128 - VK:, d:d + 1], (VK, 128)
                    )
            return _in_time_order(z)

        part_ = functools.partial
        nc = D // 256
        order = [(cols_in, 0)]
        for c in range(nc):
            order += [(cols_in, c + 1)] * (c + 1 < nc) + [(cols_out, c)]
        end = NM * R // 128
        _interleave(
            [part_(project, j, m) for j in range(R // 128) for m in reversed(range(NM))],
            ([part_(place_rows, r) for r in range(SUB, R, LR)], 0, end // 2 - 2),
            ([part_(place_rows, r) for r in range(0, SUB, LR)], end // 2, end - 1),
            ([part_(f, c, g) for f, c in order for g in range(T)], 0, end - 1),
            ([part_(f, i, n) for i in range(3) for f in (rows_in, rows_out) for n in range(16)],
             0, end - 1),
        )


@jax.jit
def pallas_interleave_layers__grouped_kv_mqa__sliding_local_dilated__prompt_kernel(
    A_x: jax.Array,
    A_wq: jax.Array,
    A_wk: jax.Array,
    A_wv: jax.Array,
    A_wo: jax.Array,
    B_x: jax.Array,
    B_wqkv: jax.Array,
    B_wo: jax.Array,
):
    del B_x
    _, S, D = A_x.shape
    NB = S // R
    T = D // 128
    vmem = pltpu.VMEM
    out = pl.pallas_call(
        _kernel,
        grid=(3 * NB,),
        in_specs=[pl.BlockSpec(memory_space=pl.ANY)] * 7,
        out_specs=pl.BlockSpec((R, D), lambda s: (jnp.maximum(s - 2 * NB, 0), 0)),
        out_shape=jax.ShapeDtypeStruct((S, D), A_x.dtype),
        scratch_shapes=[
            vmem((S, D), BF16),
            vmem((D, 5 * D), BF16),
            vmem((2, DH, D), BF16),
            vmem((T, D // 2 + DH, 128), U32),
            vmem((T * D, 128), BF16),
            vmem((4 * T, D // 2, 128), U32),
            vmem((2 * T, D // 2, 128), U32),
            vmem((2, H * PAD, 128), U32),
            vmem((H // 2 * PAD, 128), U32),
            vmem((T, S, 128), F32),
            vmem((T, R, 128), F32),
            vmem((T, R // 2, 128), U32),
            vmem((NB * D // 2, R), U32),
            vmem((DH, 128), F32),
            vmem((2, S // 2, 128), U32),
            vmem((2, S // CH, DH, VK, 128), F32),
            vmem((2, S // 128, DH // 2, 128), U32),
            vmem((HU, DH, 8, R), F32),
            vmem((CH // 2, R), U32),
            vmem((8, R), F32),
            vmem((128, R), BF16),
            vmem((T, R // 2, 128), U32),
            vmem((T, R // 2, 128), U32),
            vmem((2 * T, HALO + SUB, 128), F32),
            vmem((2 * T, HALO + SUB, 128), F32),
            vmem((T, HALO + SUB, 128), F32),
            vmem((T, HALO + SUB, 128), F32),
            vmem((W + 1, SUB, 128), F32),
            vmem((W + 1, SUB, 128), F32),
            pltpu.SemaphoreType.DMA((S // SUB + 2 * T + 6,)),
        ],
        compiler_params=pltpu.CompilerParams(
            dimension_semantics=("arbitrary",),
            vmem_limit_bytes=110 * 2**20,
        ),
        name="interleave_layers",
    )(A_x.reshape(S, D), A_wq, A_wk.T, A_wv.T, A_wo, B_wqkv, B_wo)
    return out.reshape(1, S, D)
```

```python
import functools
import math

import jax
import jax.numpy as jnp
import numpy as np
from jax import lax
from jax.experimental import pallas as pl
from jax.experimental.pallas import tpu as pltpu

F32 = jnp.float32
BF16 = jnp.bfloat16
U32 = jnp.uint32

H = 32
DH = 32
W = 8
DIL = 2
HALO = 16
EPS = 1e-5
QSCALE = DH ** -0.5 * math.log2(math.e)
MASKED = -1e9 * math.log2(math.e)

R = 512
SUB = 256
NSUB = R // SUB
VK = 16
HT4 = 128 // DH
UNITS = DH // 16 * R // 128
PAD = 33

NT = (((1,), (1,)), ((), ()))
HU = 4


def _center(xs):
    inv_d = 1.0 / (128 * len(xs))
    m = jnp.sum(functools.reduce(jnp.add, xs), axis=-1, keepdims=True) * inv_d
    ds = [x - m for x in xs]
    v = jnp.sum(functools.reduce(jnp.add, [d * d for d in ds]), axis=-1, keepdims=True) * inv_d
    return ds, lax.rsqrt(v + EPS)


def _pack(x):
    return pltpu.bitcast(x.astype(BF16), U32)


def _unpack(words):
    return pltpu.bitcast(words, BF16)


def _aligned(index, n):
    start = index * n
    return pl.ds(start if isinstance(start, int) else pl.multiple_of(start, n), n)


def _dot(a, b):
    return jnp.dot(a, b, preferred_element_type=F32)


def _lanes(tiles):
    return jnp.concatenate(tiles, axis=1)


def _tile(t):
    return slice(t * 128, (t + 1) * 128)


LEFT = (1, 2, 5, 6, 7)
RIGHT = (1, 3, 4, 6, 7)


def _left_factors(x11, x12, x21, x22):
    return x11 + x22, x21 + x22, x11 + x12, x21 - x11, x12 - x22


def _right_factors(w11, w12, w21, w22):
    return w11 + w22, w12 - w22, w21 - w11, w11 + w12, w21 + w22


def _strassen(product, emit):
    acc = {}

    def piece(n):
        y = product(n)
        if n == 2:
            acc.update(m2=y)
        elif n == 4:
            emit(1, 0, acc["m2"] + y)
            acc.update(c11=y)
        elif n == 1:
            acc.update(c11=acc["c11"] + y, c22=y - acc["m2"])
        elif n == 7:
            acc.update(c11=acc["c11"] + y)
        elif n == 5:
            emit(0, 0, acc["c11"] - y)
            acc.update(m5=y)
        elif n == 3:
            emit(0, 1, acc["m5"] + y)
            acc.update(c22=acc["c22"] + y)
        else:
            emit(1, 1, acc["c22"] + y)
        return _in_time_order(y)

    return [functools.partial(piece, n) for n in (2, 4, 1, 7, 5, 3, 6)]


def _in_time_order(y):
    return [y[r:r + 8, 0:128] for r in range(0, y.shape[0], 8)]


def _interleave(mxu, *jobs):
    todo = sorted(
        [(start + (stop - start) * i / len(pieces), j, i, piece)
         for j, (pieces, start, stop) in enumerate(jobs) for i, piece in enumerate(pieces)],
        key=lambda item: item[:3],
    )
    for n, piece in enumerate(mxu):
        results = piece()
        while todo and todo[0][0] < n + 1:
            at, _, _, other = todo.pop(0)
            other(results[int((at - n) * len(results))])
    assert not todo


def _kernel(
    x_hbm, wq_hbm, wk_hbm, wv_hbm, woa_hbm, wqkv_hbm, wob_hbm,
    o_ref,
    xin, raw, wkv, woa, wt, wqkv, wob, tmp_c, tmp_r, wt_r, w_r,
    xs, x1, oa, ln, ob, oa_l, ln_l, ob_l,
    qt, kmean, kb, kv, vt, qb, p0, l0, ot,
    lqk0, lqk1, lv0, lv1, lp0, lp1,
    sems,
):
    T, S, _ = xs.shape
    D = T * 128
    NB = S // R
    NCH = S // SUB
    HT, HS, HD = T // 2, SUB // 2, D // 2
    HWT = HD + DH
    lqk, lv, lp = (lqk0, lqk1), (lv0, lv1), (lp0, lp1)
    step = pl.program_id(0)
    is_pre = step < NB
    blk = step % NB
    row0 = pl.multiple_of(blk * R, R)
    zero = jnp.minimum(step, 0)
    true = jnp.broadcast_to(zero, (8, 128)) == 0

    def gated(x, token):
        x = jnp.broadcast_to(x, (8, 128)) if np.ndim(x) == 0 else x
        token = pltpu.bitcast(token, x.dtype)
        return jnp.concatenate(
            [jnp.where(true, x[r:r + 8], token) for r in range(0, x.shape[0], 8)], axis=0
        )

    def sub(i):
        return slice(i * SUB, (i + 1) * SUB)

    def x_copy(i):
        return pltpu.make_async_copy(x_hbm.at[sub(i)], xin.at[sub(i)], sems.at[i])

    def wq_copy(j):
        rows = pl.ds(j * 128, 128)
        return pltpu.make_async_copy(
            wq_hbm.at[rows], raw.at[rows, pl.ds(0, D)], sems.at[NCH + j]
        )

    kv_copies = [
        pltpu.make_async_copy(src, wkv.at[i], sems.at[NCH + T + i])
        for i, src in enumerate([wk_hbm, wv_hbm])
    ]
    raw_copies = [
        pltpu.make_async_copy(src, raw.at[:, pl.ds((i + 1) * D, D)], sems.at[NCH + T + 2 + i])
        for i, src in enumerate([wqkv_hbm.at[:, pl.ds(p * D, D)] for p in range(3)] + [wob_hbm])
    ]
    woa_copies = [
        pltpu.make_async_copy(
            woa_hbm.at[:, _tile(t)], woa.at[pl.ds(t * D, D)], sems.at[NCH + T + 6 + t]
        )
        for t in range(T)
    ]

    def load_x(g):
        x = xin[_aligned(g, 16), :].astype(F32)
        return [x[:, _tile(t)] for t in range(T)]

    def store_norm(g, x):
        ds, inv = _center(x)
        ln[_aligned(g, 8), :] = _pack(_lanes(ds) * inv)

    def store_left_factors(src, dst, i, r, c):
        ys = _left_factors(*[
            _unpack(src[pl.ds((i * SUB + y) // 2, 8), pl.ds(z + c * 256, 256)]).astype(F32)
            for y in (r, HS + r) for z in (0, HD)
        ])
        for n, y in enumerate(ys):
            dst[pl.ds(((i * 5 + n) * HS + r) // 2, 8), pl.ds(c * 256, 256)] = _pack(y)

    def left_factor(src, dst, i, n):
        if n in LEFT:
            return _unpack(dst[_aligned(i * 5 + LEFT.index(n), HS // 2), :])
        half = n - 3
        return _unpack(src[pl.ds((i * SUB + half * HS) // 2, HS // 2), pl.ds(half * HD, HD)])

    def weight(m, t, half, part=0, parts=1):
        n = HD // parts
        if m == 0:
            return woa[_aligned((2 * t + half) * parts + part, n), :]
        rows = _aligned(half * parts + part, n // 2)
        return _unpack(wob[T + t, rows, :] if m == 4 else wqkv[m * T + t, rows, :])

    def right_factor(m, n, t):
        if n in RIGHT:
            return _unpack(w_r[_aligned(m * 5 + RIGHT.index(n), HD // 2), _tile(t)])
        return weight(m, t + (n == 5) * HT, int(n == 5))

    @pl.when(step == 0)
    def _():
        ahead, n = 4, 2
        x_copy(0).start()
        for j in range(ahead):
            wq_copy(j).start()
        for c in kv_copies:
            c.start()
        lqk1[:, SUB:, :] = jnp.zeros((2 * T, HALO, 128), F32)
        lv1[:, SUB:, :] = jnp.zeros((T, HALO, 128), F32)
        ot[...] = jnp.zeros(ot.shape, BF16)
        kmean[...] = jnp.zeros(kmean.shape, F32)
        x1[...] = jnp.zeros(x1.shape, F32)
        x_copy(0).wait()

        def first_rows(i, _):
            for u in range(n):
                j = i * n + u
                pl.when(j + ahead < T)(wq_copy(jnp.minimum(j + ahead, T - 1)).start)
                pl.when(j + ahead == T)(x_copy(1).start)
                pl.when(j + ahead == T + 1)(x_copy(2).start)
                wq_copy(j).wait()
            for u in range(n):
                j = i * n + u
                wt[pl.ds(pl.multiple_of(j * HWT, 8), HD), :] = _pack(raw[_aligned(j, 128), 0:D].T)
                for g in range(SUB // T // 16):
                    g = j * (SUB // T // 16) + g
                    store_norm(g, load_x(g))

        lax.fori_loop(0, T // n, first_rows, None)
        for i, c in enumerate(kv_copies):
            c.wait()
            for j in range(T):
                wt[pl.ds(j * HWT + (D + i * DH) // 2, DH // 2), :] = pltpu.bitcast(wkv[i, :, _tile(j)], U32)

        for c in range(HT // 2):
            def wt_factors(r, _):
                ys = _right_factors(*[
                    _lanes([
                        _unpack(wt[_aligned(((k + 2 * c + u) * 2 + y) * (HWT // 16) + r, 8), :]).astype(F32)
                        for u in range(2)
                    ])
                    for k in (0, HT) for y in range(2)
                ])
                for j, y in enumerate(ys):
                    wt_r[_aligned(j * (HWT // 16) + r, 8), pl.ds(c * 256, 256)] = _pack(y)

            lax.fori_loop(0, HWT // 16, wt_factors, None, unroll=2)
            for r in range(0, HS, 16):
                store_left_factors(ln, ln_l, 0, r, c)

    for s, waits, starts in ((0, (), (0, 3)), (1, (0, 3), (1,)), (2, (1,), (2,)), (3, (2,), ())):
        @pl.when(step == s)
        def _():
            for i in range(NSUB * s + 1, min(NSUB * (s + 1) + 1, NCH)):
                x_copy(i).wait()
            for i in waits:
                raw_copies[i].wait()
            for i in range(NSUB * (s + 1) + 1, min(NSUB * (s + 2) + 1, NCH)):
                x_copy(i).start()
            for i in starts:
                raw_copies[i].start()
            if s == NB - 1:
                for c in woa_copies:
                    c.start()

    @pl.when(step == NB)
    def _():
        for c in woa_copies:
            c.wait()

        def w_factors(i, _):
            c, part = i // 16, i % 16
            for m in range(5):
                ys = _right_factors(*[
                    _lanes([weight(m, k + 2 * c + u, half, part, 16).astype(F32) for u in range(2)])
                    for half in range(2) for k in (0, HT)
                ])
                for j, y in enumerate(ys):
                    w_r[_aligned((m * 5 + j) * 16 + part, HD // 32), _aligned(c, 256)] = _pack(y)

        lax.fori_loop(0, HT // 2 * 16, w_factors, None)

    @pl.when(step == 2 * NB)
    def _():
        for ref in (kb, vt):
            half = ref.shape[0] // 2
            n = half // NB * (NB - 1)
            ref[0:n] = ref[half:half + n]
        n = NSUB * (NB - 1)
        kv[0, 0:n] = kv[1, 0:n]

    @pl.when(step >= NB)
    def _():
        def q_rows(h):
            return jnp.minimum(blk * H + h, NB * H - 1)

        def load_q(h):
            q = _unpack(qt[_aligned(q_rows(h), DH // 2), :])
            return jnp.concatenate([q, jnp.zeros((128 - DH, R), BF16)], axis=0)

        def spread_q(h, slot, unit, token):
            g, cols = unit // (R // 128), _tile(unit % (R // 128))
            w = qt[_aligned(q_rows(h) * (DH // 16) + g, 8), cols]
            if token is not None:
                w = gated(w, token)
            for odd, y in enumerate((w << 16, w & np.uint32(0xFFFF0000))):
                y = pltpu.bitcast(y, F32)
                for i in range(8):
                    qb[slot, 16 * g + 2 * i + odd, :, cols] = jnp.broadcast_to(y[i:i + 1], (8, 128))

        def scores(q, c):
            return _dot(_unpack(kb[pl.ds(c * SUB // 2, (SUB - VK) // 2), :]), q)

        def probs(s, slot, c, tokens):
            rest = None
            for d in range(DH):
                k = kv[0, c, d]
                if d % 2 == 0:
                    k = gated(k, tokens[d * len(tokens) // DH])
                y = _lanes([k] * (R // 128)) * jnp.concatenate([qb[slot, d]] * (VK // 8), axis=0)
                rest = y if rest is None else rest + y
            p = jnp.exp2(jnp.concatenate([s, rest], axis=0))
            return p.astype(BF16), p.reshape(SUB // 8, 8, R).sum(axis=0)

        @pl.when(blk == 0)
        def _():
            for unit in range(UNITS):
                spread_q(0, 0, unit, None)
            s = scores(load_q(0), 0)
            p, l = probs(s, 0, 0, _in_time_order(s)[:1])
            p0[...] = pltpu.bitcast(p, U32)
            l0[...] = l

        def fast_heads(it, carry):
            low, every = carry
            qs = [load_q(it * HU + u) for u in range(HU + 1)]
            p, l = _unpack(p0[...]), l0[...]
            for u in range(HU):
                acc = None
                for c in range(NCH):
                    v, c2 = u + (c + 1) // NCH, (c + 1) % NCH
                    s = scores(qs[v], c2)
                    pv = _dot(_unpack(vt[_aligned(c, DH // 2), :]), p)
                    acc = pv if acc is None else acc + pv
                    tokens = _in_time_order(s) + _in_time_order(pv)
                    p, l_next = probs(s, v % HT4, c2, tokens)
                    if c2:
                        l = l + l_next
                        units = range(c * UNITS // (NCH - 1), c2 * UNITS // (NCH - 1))
                        for i, unit in enumerate(units):
                            spread_q(it * HU + u + 1, (u + 1) % HT4, unit, tokens[-1 - 15 * i])
                    if u % HT4 == 0 and c == 2:
                        w = pltpu.bitcast(ot[...], U32)
                        w = _lanes([gated(w[:, _tile(j)], tokens[0]) for j in range(R // 128)])
                        oa[:, _aligned(((it * HU + u) // HT4 + T - 1) % T, 128)] = _pack(_unpack(w).T)
                total = jnp.sum(l, axis=0, keepdims=True)
                l = l_next
                ot[_aligned(u % HT4, DH), :] = (acc * (1.0 / total)).astype(BF16)
                low = jnp.minimum(low, total)
                every = every + acc.reshape(DH // 8, 8, R).sum(axis=0) + total
            p0[...] = pltpu.bitcast(p, U32)
            l0[...] = l
            return low, every

        low, every = lax.fori_loop(
            0, H // HU, fast_heads, (jnp.ones((1, R), F32), jnp.zeros((8, R), F32))
        )

        def safe_heads():
            def safe_tile(tile, _):
                def safe_head(u, _):
                    q = load_q(tile * HT4 + u)

                    def chunk(c, carry):
                        m, l, acc = carry
                        s = _dot(_unpack(kb[_aligned(c, SUB // 2), :]), q)
                        m_new = jnp.maximum(m, jnp.max(s, axis=0, keepdims=True))
                        alpha = jnp.exp2(m - m_new)
                        p = jnp.exp2(s - m_new)
                        l = alpha * l + jnp.sum(p, axis=0, keepdims=True)
                        acc = alpha * acc + _dot(_unpack(vt[_aligned(c, DH // 2), :]), p.astype(BF16))
                        return m_new, l, acc

                    init = (
                        jnp.full((1, R), -jnp.inf, F32),
                        jnp.zeros((1, R), F32),
                        jnp.zeros((DH, R), F32),
                    )
                    _, l, acc = lax.fori_loop(0, NCH, chunk, init)
                    ot[_aligned(u, DH), :] = (acc / l).astype(BF16)

                lax.fori_loop(0, HT4, safe_head, None)
                oa[:, _aligned(tile, 128)] = _pack(ot[...].T)

            lax.fori_loop(0, T, safe_tile, None)

        @pl.when(zero == 0)
        def _():
            oa[:, _tile(T - 1)] = _pack(ot[...].T)
            ok = jnp.where(jnp.logical_and(low >= 1.0, jnp.abs(every) < 3e38), 1.0, 0.0)
            pl.when(jnp.min(ok) < 1.0)(safe_heads)

        first = blk == 0

        def project(src, dst, i, m, emit):
            return [
                piece for t in range(HT) for piece in _strassen(
                    lambda n, t=t: _dot(left_factor(src, dst, i, n), right_factor(m, n, t)),
                    lambda r, c, y, t=t: emit(r * HS, c * HT + t, y),
                )
            ]

        def combine(src, dst, i, r):
            return [
                lambda _, c=c: store_left_factors(src, dst, i, r, c) for c in range(HT // 2)
            ]

        def row_stage(rows, src, dst, i):
            held = []

            def piece(r, token):
                ys, scale = rows(r, token)
                held.append(_lanes([y * scale for y in ys]))
                if len(held) == 2:
                    src[pl.ds((i * SUB + r - 8) // 2, 8), :] = _pack(jnp.concatenate(held, axis=0))
                    held.clear()

            pieces = []
            for r in range(0, HS, 16):
                pieces += [functools.partial(piece, y) for y in (r, r + 8, HS + r, HS + r + 8)]
                if r:
                    pieces += combine(src, dst, i, r - 16)
            return pieces + combine(src, dst, i, HS - 16)

        def out_proj_a(i):
            def emit(r, t, y):
                rows = _aligned((blk * NSUB + i) * 2 + r // HS, HS)
                y = y + xs[t, rows, :]
                x1[t, pl.ds(i * SUB + r, HS), :] = y

            return project(oa, oa_l, i, 0, emit)

        def combine_a(i):
            return [piece for r in range(0, HS, 16) for piece in combine(oa, oa_l, i, r)]

        def norm(i):
            def rows(r, token):
                x = [x1[t, pl.ds(i * SUB + r, 8), :] for t in range(T)]
                return _center([gated(x[0], token)] + x[1:])

            return row_stage(rows, ln, ln_l, i)

        def qkv_proj(i, part):
            def emit(r, t, z):
                if part == 0:
                    lqk[i][t, pl.ds(HALO + r, HS), :] = z
                    return
                refs, t = (lqk, T + t) if part == 1 else (lv, t)
                if i == 0 and r == 0:
                    refs[0][t, 0:HALO, :] = jnp.where(first, z[0:1, :], refs[-1][t, SUB:, :])
                if i + 1 < NSUB and r:
                    refs[i + 1][t, 0:HALO, :] = z[HS - HALO:, :]
                refs[i][t, pl.ds(HALO + r, HS), :] = z

            return project(ln, ln_l, i, part + 1, emit)

        def window(r, w):
            return pl.ds(HALO + r - DIL * w, 8)

        def local_probs(i):
            def piece(r, token):
                scale = gated(np.float32(QSCALE), token)
                q = [lqk[i][t, window(r, 0), :] * scale for t in range(T)]
                z = []
                for w in range(W):
                    y = functools.reduce(jnp.add, [
                        q[t] * lqk[i][T + t, window(r, w), :] for t in range(T)
                    ])
                    y = y + pltpu.roll(y, 2 * H, 1)
                    y = y + pltpu.roll(y, H, 1)
                    if i == 0 and r < DIL * w:
                        pos = row0 + r + lax.broadcasted_iota(jnp.int32, (8, 128), 0)
                        y = jnp.where(pos >= DIL * w, y, MASKED)
                    z.append(y)
                m = functools.reduce(jnp.maximum, z)
                e = [jnp.exp2(y - m) for y in z]
                for w in range(W):
                    lp[i][w, r:r + 8, :] = e[w]
                lp[i][W, r:r + 8, :] = 1.0 / functools.reduce(jnp.add, e)

            return [functools.partial(piece, r) for r in range(0, SUB, 8)]

        def local_values(i):
            def rows(r, token):
                p = [gated(lp[i][w, r:r + 8, :], token) for w in range(W)]
                return [
                    functools.reduce(jnp.add, [p[w] * lv[i][t, window(r, w), :] for w in range(W)])
                    for t in range(T)
                ], lp[i][W, r:r + 8, :]

            return row_stage(rows, ob, ob_l, i)

        def out_proj_b(i):
            def emit(r, t, y):
                rows = pl.ds(i * SUB + r, HS)
                y = y + x1[t, rows, :]
                x1[t, rows, :] = y
                o_ref[rows, _tile(t)] = y.astype(BF16)

            return project(ob, ob_l, i, 4, emit)

        Q, K, V = range(3)
        for piece in combine_a(0):
            piece(None)
        _interleave(out_proj_a(0), (combine_a(1), 0, 25))
        _interleave(out_proj_a(1), (norm(0), 0, 25))
        _interleave(qkv_proj(0, K) + qkv_proj(0, Q), (norm(1), 0, 45))
        _interleave(qkv_proj(1, K) + qkv_proj(1, Q), (local_probs(0), 0, 52))
        _interleave(qkv_proj(0, V), (local_probs(1), 0, 26))
        _interleave(qkv_proj(1, V), (local_values(0), 0, 24))
        _interleave(out_proj_b(0), (local_values(1), 0, 21))
        _interleave(out_proj_b(1), (norm(0), 0, 24))

    @pl.when(step < 2 * NB)
    def _():
        slot = jnp.where(jnp.logical_and(step >= NB, blk < NB - 1), 1, 0)
        part = jnp.where(is_pre, step, 0)

        def cols_in(c, g, token):
            w = pltpu.bitcast(raw[sub(c), _aligned(part * T + g, 128)], U32)
            w = jnp.concatenate([gated(w[:8], token), w[8:]], axis=0).T
            for u in range(4):
                tmp_c[c, pl.ds((4 * g + u) * PAD, DH), :] = w[u * DH:(u + 1) * DH]

        def cols_out(c, g, token):
            w = jnp.concatenate(
                [tmp_c[c, pl.ds(4 * g + u, H, stride=PAD), :] for u in range(4)], axis=0
            )
            w = jnp.concatenate([gated(w[:8], token), w[8:]], axis=0)
            wqkv[part * T + g, _tile(c), :] = w.T

        def wob_tile(i):
            j = jnp.where(part > 0, jnp.minimum(T + 3 * (part - 1) + i, 2 * T - 1), i)
            return j, jnp.where(part > 0, 3 * T + j, j)

        def rows_in(i, n, token):
            w = raw[_aligned(n, 2 * DH), _aligned(wob_tile(i)[1], 128)]
            tmp_r[pl.ds(n * PAD, DH), :] = gated(pltpu.bitcast(w, U32), token)

        def rows_out(i, e, token):
            low = jnp.concatenate([gated(np.uint32(0xFFFF), token)] * 2, axis=0)
            a = tmp_r[pl.ds(e, H // 2, stride=PAD), :]
            b = tmp_r[pl.ds(DH // 2 + e, H // 2, stride=PAD), :]
            even = (a & low) | (b << 16)
            odd = (a >> 16) | (b & ~low)
            wob[wob_tile(i)[0], _aligned(e, H), :] = jnp.concatenate([even, odd], axis=0)

        def place_rows(g, token):
            mask = jnp.concatenate([jnp.logical_and(true, is_pre)] * 2, axis=0)
            x = [
                jnp.where(mask, y, gated(x1[t, _aligned(g, 16), :], token))
                for t, y in enumerate(load_x(blk * (R // 16) + g))
            ]
            for t in range(T):
                xs[t, _aligned(blk * (R // 16) + g, 16), :] = x[t]
            if g < SUB // 16:
                x = [gated(y, token) for y in load_x((blk + 1) % NB * (R // 16) + g)]
            store_norm(g, x)

        def place(i):
            pieces = []
            for r in range(0, HS, 16):
                pieces += [functools.partial(place_rows, (i * SUB + y) // 16) for y in (r, HS + r)]
                pieces += [
                    lambda _, r=r, c=c: store_left_factors(ln, ln_l, i, r, c) for c in range(HT // 2)
                ]
            return pieces

        def project(i, r, size):
            def product(n):
                if n in RIGHT:
                    w = wt_r[pl.ds((RIGHT.index(n) * HWT + r) // 2, size // 2), :]
                else:
                    start = ((n == 5) * HWT + r) // 2
                    w = _lanes([
                        wt[pl.ds(((n == 5) * HT + t) * HWT + start, size // 2), :] for t in range(HT)
                    ])
                return lax.dot_general(
                    _unpack(w), left_factor(ln, ln_l, i, n), NT, preferred_element_type=F32
                )

            held = {}

            def pair(a, b, z):
                if b in held:
                    emit(i, b * HWT + r, _lanes([held.pop(b), z] if a else [z, held.pop(b)]))
                else:
                    held[b] = z

            return _strassen(product, pair)

        def emit(i, r, z):
            nq = min(len(z), D - r)
            rows = pl.ds(pl.multiple_of(blk * (D // 2) + r // 2, 8), nq // 2)
            qt[rows, sub(i)] = _pack(z[:nq])
            if nq == len(z):
                return
            n = blk * NSUB + i
            vt[_aligned(slot * NCH + n, DH // 2), :] = _pack(z[nq + DH:])
            k = z[nq:nq + DH]
            if i == 0:
                mean = jnp.sum(k[:, :128], axis=-1, keepdims=True) * (1.0 / 128)
                kmean[...] = jnp.where(jnp.broadcast_to(blk, (DH, 128)) == 0, mean, kmean[...])
            k = (k - _lanes([kmean[...]] * (SUB // 128))) * QSCALE
            k = jnp.concatenate([k, jnp.zeros((128 - DH, SUB), F32)], axis=0).T
            kb[_aligned(slot * NCH + n, SUB // 2), :] = _pack(k)
            for d in range(DH):
                kv[slot, n, d] = jnp.broadcast_to(k[SUB - VK:, d:d + 1], (VK, 128))

        chunks = [(384, 160), (192, 192), (0, 192)]
        assert sum(chunks[0]) == HWT
        order = [(f, c) for f in (cols_in, cols_out) for c in range(D // SUB)]
        end = 7 * len(chunks) * NSUB
        _interleave(
            [piece for i in range(NSUB) for chunk in chunks for piece in project(i, *chunk)],
            (place(1), 0, end // 2 - 3),
            (place(0), end // 2, end - 2),
            ([functools.partial(f, c, g) for f, c in order for g in range(T)], 0, end - 5),
            ([functools.partial(f, i, n)
              for i in range(3) for f in (rows_in, rows_out) for n in range(16)], 0, end - 1),
        )


@jax.jit
def pallas_interleave_layers__grouped_kv_mqa__sliding_local_dilated__prompt_kernel(
    A_x: jax.Array,
    A_wq: jax.Array,
    A_wk: jax.Array,
    A_wv: jax.Array,
    A_wo: jax.Array,
    B_x: jax.Array,
    B_wqkv: jax.Array,
    B_wo: jax.Array,
):
    del B_x
    _, S, D = A_x.shape
    NB = S // R
    T = D // 128
    vmem = pltpu.VMEM
    left = vmem((NSUB * 5 * SUB // 4, D // 2), U32)
    out = pl.pallas_call(
        _kernel,
        grid=(3 * NB,),
        in_specs=[pl.BlockSpec(memory_space=pl.ANY)] * 7,
        out_specs=pl.BlockSpec((R, D), lambda s: (jnp.maximum(s - 2 * NB, 0), 0)),
        out_shape=jax.ShapeDtypeStruct((S, D), A_x.dtype),
        scratch_shapes=[
            vmem((S, D), BF16),
            vmem((D, 5 * D), BF16),
            vmem((2, DH, D), BF16),
            vmem((T * D, 128), BF16),
            vmem((T * (D // 2 + DH), 128), U32),
            vmem((4 * T, D // 2, 128), U32),
            vmem((2 * T, D // 2, 128), U32),
            vmem((D // SUB, H * PAD, 128), U32),
            vmem((H // 2 * PAD, 128), U32),
            vmem((5 * (D // 2 + DH) // 2, D // 2), U32),
            vmem((5 * 5 * D // 4, D // 2), U32),
            vmem((T, S, 128), F32),
            vmem((T, R, 128), F32),
            vmem((R // 2, D), U32),
            vmem((R // 2, D), U32),
            vmem((R // 2, D), U32),
            left,
            left,
            left,
            vmem((NB * D // 2, R), U32),
            vmem((DH, 128), F32),
            vmem((2 * S // 2, 128), U32),
            vmem((2, S // SUB, DH, VK, 128), F32),
            vmem((2 * S // SUB * DH // 2, SUB), U32),
            vmem((HT4, DH, 8, R), F32),
            vmem((SUB // 2, R), U32),
            vmem((8, R), F32),
            vmem((128, R), BF16),
            vmem((2 * T, HALO + SUB, 128), F32),
            vmem((2 * T, HALO + SUB, 128), F32),
            vmem((T, HALO + SUB, 128), F32),
            vmem((T, HALO + SUB, 128), F32),
            vmem((W + 1, SUB, 128), F32),
            vmem((W + 1, SUB, 128), F32),
            pltpu.SemaphoreType.DMA((S // SUB + 2 * T + 6,)),
        ],
        compiler_params=pltpu.CompilerParams(
            dimension_semantics=("arbitrary",),
            vmem_limit_bytes=120 * 2**20,
        ),
        name="interleave_layers",
    )(A_x.reshape(S, D), A_wq, A_wk.T, A_wv.T, A_wo, B_wqkv, B_wo)
    return out.reshape(1, S, D)
```

```python
import functools
import math

import jax
import jax.numpy as jnp
import numpy as np
from jax import lax
from jax.experimental import pallas as pl
from jax.experimental.pallas import tpu as pltpu

F32 = jnp.float32
BF16 = jnp.bfloat16
U32 = jnp.uint32

H = 32
DH = 32
W = 8
DIL = 2
HALO = 16
EPS = 1e-5
QSCALE = DH ** -0.5 * math.log2(math.e)
MASKED = -1e9 * math.log2(math.e)

R = 512
SUB = 256
NSUB = R // SUB
VK = 16
HT4 = 128 // DH
UNITS = DH // 16 * R // 128
PAD = 33

NT = (((1,), (1,)), ((), ()))
HU = 8


def _center(xs):
    inv_d = 1.0 / (128 * len(xs))
    m = jnp.sum(functools.reduce(jnp.add, xs), axis=-1, keepdims=True) * inv_d
    ds = [x - m for x in xs]
    v = jnp.sum(functools.reduce(jnp.add, [d * d for d in ds]), axis=-1, keepdims=True) * inv_d
    return ds, lax.rsqrt(v + EPS)


def _pack(x):
    return pltpu.bitcast(x.astype(BF16), U32)


def _unpack(words):
    return pltpu.bitcast(words, BF16)


def _aligned(index, n):
    start = index * n
    return pl.ds(start if isinstance(start, int) else pl.multiple_of(start, n), n)


def _dot(a, b):
    return jnp.dot(a, b, preferred_element_type=F32)


def _lanes(tiles):
    return jnp.concatenate(tiles, axis=1)


def _tile(t):
    return slice(t * 128, (t + 1) * 128)


LEFT = (1, 2, 5, 6, 7)
RIGHT = (1, 3, 4, 6, 7)


def _left_factors(x11, x12, x21, x22):
    return x11 + x22, x21 + x22, x11 + x12, x21 - x11, x12 - x22


def _right_factors(w11, w12, w21, w22):
    return w11 + w22, w12 - w22, w21 - w11, w11 + w12, w21 + w22


def _strassen(product, emit):
    acc = {}

    def piece(n):
        y = product(n)
        if n == 2:
            acc.update(m2=y)
        elif n == 4:
            emit(1, 0, acc["m2"] + y)
            acc.update(c11=y)
        elif n == 1:
            acc.update(c11=acc["c11"] + y, c22=y - acc["m2"])
        elif n == 7:
            acc.update(c11=acc["c11"] + y)
        elif n == 5:
            emit(0, 0, acc["c11"] - y)
            acc.update(m5=y)
        elif n == 3:
            emit(0, 1, acc["m5"] + y)
            acc.update(c22=acc["c22"] + y)
        else:
            emit(1, 1, acc["c22"] + y)
        return _in_time_order(y)

    return [functools.partial(piece, n) for n in (2, 4, 1, 7, 5, 3, 6)]


def _in_time_order(y):
    return [y[r:r + 8, 0:128] for r in range(0, y.shape[0], 8)]


def _interleave(mxu, *jobs):
    todo = sorted(
        [(start + (stop - start) * i / len(pieces), j, i, piece)
         for j, (pieces, start, stop) in enumerate(jobs) for i, piece in enumerate(pieces)],
        key=lambda item: item[:3],
    )
    for n, piece in enumerate(mxu):
        results = piece()
        while todo and todo[0][0] < n + 1:
            at, _, _, other = todo.pop(0)
            other(results[int((at - n) * len(results))])
    assert not todo


def _kernel(
    x_hbm, wq_hbm, wk_hbm, wv_hbm, woa_hbm, wqkv_hbm, wob_hbm,
    o_ref,
    xin, raw, wkv, woa, wt, wqkv, wob, tmp_c, tmp_r, wt_r, w_r,
    xs, x1, oa, ln, ob, oa_l, ln_l, ob_l,
    qt, kmean, kb, kv, vt, qb, p0, l0, ot,
    lqk0, lqk1, lv0, lv1, lp0, lp1,
    sems,
):
    T, S, _ = xs.shape
    D = T * 128
    NB = S // R
    NCH = S // SUB
    HT, HS, HD = T // 2, SUB // 2, D // 2
    HWT = HD + DH
    lqk, lv, lp = (lqk0, lqk1), (lv0, lv1), (lp0, lp1)
    step = pl.program_id(0)
    is_pre = step < NB
    blk = step % NB
    row0 = pl.multiple_of(blk * R, R)
    zero = jnp.minimum(step, 0)
    true = jnp.broadcast_to(zero, (8, 128)) == 0

    def gated(x, token):
        x = jnp.broadcast_to(x, (8, 128)) if np.ndim(x) == 0 else x
        token = pltpu.bitcast(token, x.dtype)
        return jnp.concatenate(
            [jnp.where(true, x[r:r + 8], token) for r in range(0, x.shape[0], 8)], axis=0
        )

    def sub(i):
        return slice(i * SUB, (i + 1) * SUB)

    def x_copy(i):
        return pltpu.make_async_copy(x_hbm.at[sub(i)], xin.at[sub(i)], sems.at[i])

    def wq_copy(j):
        rows = pl.ds(j * 128, 128)
        return pltpu.make_async_copy(
            wq_hbm.at[rows], raw.at[rows, pl.ds(0, D)], sems.at[NCH + j]
        )

    kv_copies = [
        pltpu.make_async_copy(src, wkv.at[i], sems.at[NCH + T + i])
        for i, src in enumerate([wk_hbm, wv_hbm])
    ]
    raw_copies = [
        pltpu.make_async_copy(src, raw.at[:, pl.ds((i + 1) * D, D)], sems.at[NCH + T + 2 + i])
        for i, src in enumerate([wqkv_hbm.at[:, pl.ds(p * D, D)] for p in range(3)] + [wob_hbm])
    ]
    woa_copies = [
        pltpu.make_async_copy(
            woa_hbm.at[:, _tile(t)], woa.at[pl.ds(t * D, D)], sems.at[NCH + T + 6 + t]
        )
        for t in range(T)
    ]

    def load_x(g):
        x = xin[_aligned(g, 16), :].astype(F32)
        return [x[:, _tile(t)] for t in range(T)]

    def store_norm(g, x):
        ds, inv = _center(x)
        ln[_aligned(g, 8), :] = _pack(_lanes(ds) * inv)

    def store_left_factors(src, dst, i, r, c):
        ys = _left_factors(*[
            _unpack(src[pl.ds((i * SUB + y) // 2, 8), pl.ds(z + c * 256, 256)]).astype(F32)
            for y in (r, HS + r) for z in (0, HD)
        ])
        for n, y in enumerate(ys):
            dst[pl.ds(((i * 5 + n) * HS + r) // 2, 8), pl.ds(c * 256, 256)] = _pack(y)

    def left_factor(src, dst, i, n):
        if n in LEFT:
            return _unpack(dst[_aligned(i * 5 + LEFT.index(n), HS // 2), :])
        half = n - 3
        return _unpack(src[pl.ds((i * SUB + half * HS) // 2, HS // 2), pl.ds(half * HD, HD)])

    def weight(m, t, half, part=0, parts=1):
        n = HD // parts
        if m == 0:
            return woa[_aligned((2 * t + half) * parts + part, n), :]
        rows = _aligned(half * parts + part, n // 2)
        return _unpack(wob[T + t, rows, :] if m == 4 else wqkv[m * T + t, rows, :])

    def right_factor(m, n, t):
        if n in RIGHT:
            return _unpack(w_r[_aligned(m * 5 + RIGHT.index(n), HD // 2), _tile(t)])
        return weight(m, t + (n == 5) * HT, int(n == 5))

    @pl.when(step == 0)
    def _():
        ahead, n = 4, 2
        x_copy(0).start()
        for j in range(ahead):
            wq_copy(j).start()
        for c in kv_copies:
            c.start()
        lqk1[:, SUB:, :] = jnp.zeros((2 * T, HALO, 128), F32)
        lv1[:, SUB:, :] = jnp.zeros((T, HALO, 128), F32)
        ot[...] = jnp.zeros(ot.shape, BF16)
        kmean[...] = jnp.zeros(kmean.shape, F32)

        @pl.loop(0, T)
        def _(t):
            x1[t] = jnp.zeros((R, 128), F32)

        x_copy(0).wait()

        def first_rows(i, _):
            for u in range(n):
                j = i * n + u
                pl.when(j + ahead < T)(wq_copy(jnp.minimum(j + ahead, T - 1)).start)
                pl.when(j + ahead == T)(x_copy(1).start)
                pl.when(j + ahead == T + 1)(x_copy(2).start)
                wq_copy(j).wait()
            for u in range(n):
                j = i * n + u
                wt[pl.ds(pl.multiple_of(j * HWT, 8), HD), :] = _pack(raw[_aligned(j, 128), 0:D].T)
                for g in range(SUB // T // 16):
                    g = j * (SUB // T // 16) + g
                    store_norm(g, load_x(g))

        lax.fori_loop(0, T // n, first_rows, None)
        for i, c in enumerate(kv_copies):
            c.wait()
            for j in range(T):
                wt[pl.ds(j * HWT + (D + i * DH) // 2, DH // 2), :] = pltpu.bitcast(wkv[i, :, _tile(j)], U32)

        for c in range(HT // 2):
            def wt_factors(r, _):
                ys = _right_factors(*[
                    _lanes([
                        _unpack(wt[_aligned(((k + 2 * c + u) * 2 + y) * (HWT // 16) + r, 8), :]).astype(F32)
                        for u in range(2)
                    ])
                    for k in (0, HT) for y in range(2)
                ])
                for j, y in enumerate(ys):
                    wt_r[_aligned(j * (HWT // 16) + r, 8), pl.ds(c * 256, 256)] = _pack(y)

            lax.fori_loop(0, HWT // 16, wt_factors, None, unroll=2)
            for r in range(0, HS, 16):
                store_left_factors(ln, ln_l, 0, r, c)

    for s, waits, starts in ((0, (), (0, 3)), (1, (0, 3), (1,)), (2, (1,), (2,)), (3, (2,), ())):
        @pl.when(step == s)
        def _():
            for i in range(NSUB * s + 1, min(NSUB * (s + 1) + 1, NCH)):
                x_copy(i).wait()
            for i in waits:
                raw_copies[i].wait()
            for i in range(NSUB * (s + 1) + 1, min(NSUB * (s + 2) + 1, NCH)):
                x_copy(i).start()
            for i in starts:
                raw_copies[i].start()
            if s == NB - 1:
                for c in woa_copies:
                    c.start()

    @pl.when(step == NB)
    def _():
        for c in woa_copies:
            c.wait()

        def w_factors(i, _):
            c, part = i // 16, i % 16
            for m in range(5):
                ys = _right_factors(*[
                    _lanes([weight(m, k + 2 * c + u, half, part, 16).astype(F32) for u in range(2)])
                    for half in range(2) for k in (0, HT)
                ])
                for j, y in enumerate(ys):
                    w_r[_aligned((m * 5 + j) * 16 + part, HD // 32), _aligned(c, 256)] = _pack(y)

        lax.fori_loop(0, HT // 2 * 16, w_factors, None)

    @pl.when(step == 2 * NB)
    def _():
        for ref in (kb, vt):
            half = ref.shape[0] // 2
            n = half // NB * (NB - 1)
            ref[0:n] = ref[half:half + n]

        @pl.loop(0, NSUB * (NB - 1))
        def _(c):
            kv[0, c] = kv[1, c]


    @pl.when(step >= NB)
    def _():
        def q_rows(h):
            return jnp.minimum(blk * H + h, NB * H - 1)

        def load_q(h):
            q = _unpack(qt[_aligned(q_rows(h), DH // 2), :])
            return jnp.concatenate([q, jnp.zeros((128 - DH, R), BF16)], axis=0)

        def spread_q(h, slot, unit, token):
            g, cols = unit // (R // 128), _tile(unit % (R // 128))
            w = qt[_aligned(q_rows(h) * (DH // 16) + g, 8), cols]
            if token is not None:
                w = gated(w, token)
            for odd, y in enumerate((w << 16, w & np.uint32(0xFFFF0000))):
                y = pltpu.bitcast(y, F32)
                for i in range(8):
                    qb[slot, 16 * g + 2 * i + odd, :, cols] = jnp.broadcast_to(y[i:i + 1], (8, 128))

        def scores(q, c):
            return _dot(_unpack(kb[pl.ds(c * SUB // 2, (SUB - VK) // 2), :]), q)

        def probs(s, slot, c, tokens):
            rest = None
            for d in range(DH):
                k = kv[0, c, d]
                if d % 2 == 0:
                    k = gated(k, tokens[d * len(tokens) // DH])
                y = _lanes([k] * (R // 128)) * jnp.concatenate([qb[slot, d]] * (VK // 8), axis=0)
                rest = y if rest is None else rest + y
            p = jnp.exp2(jnp.concatenate([s, rest], axis=0))
            return p.astype(BF16), p.reshape(SUB // 8, 8, R).sum(axis=0)

        @pl.when(blk == 0)
        def _():
            for unit in range(UNITS):
                spread_q(0, 0, unit, None)
            s = scores(load_q(0), 0)
            p, l = probs(s, 0, 0, _in_time_order(s)[:1])
            p0[...] = pltpu.bitcast(p, U32)
            l0[...] = l

        def fast_heads(it, carry):
            low, every = carry
            qs = [load_q(it * HU + u) for u in range(HU + 1)]
            p, l = _unpack(p0[...]), l0[...]
            for u in range(HU):
                acc = None
                for c in range(NCH):
                    v, c2 = u + (c + 1) // NCH, (c + 1) % NCH
                    s = scores(qs[v], c2)
                    pv = _dot(_unpack(vt[_aligned(c, DH // 2), :]), p)
                    acc = pv if acc is None else acc + pv
                    tokens = _in_time_order(s) + _in_time_order(pv)
                    p, l_next = probs(s, v % HT4, c2, tokens)
                    if c2:
                        l = l + l_next
                        units = range(c * UNITS // (NCH - 1), c2 * UNITS // (NCH - 1))
                        for i, unit in enumerate(units):
                            spread_q(it * HU + u + 1, (u + 1) % HT4, unit, tokens[-1 - 15 * i])
                    if u % HT4 == 0 and c == 2:
                        w = pltpu.bitcast(ot[...], U32)
                        w = _lanes([gated(w[:, _tile(j)], tokens[0]) for j in range(R // 128)])
                        oa[:, _aligned(((it * HU + u) // HT4 + T - 1) % T, 128)] = _pack(_unpack(w).T)
                total = jnp.sum(l, axis=0, keepdims=True)
                l = l_next
                ot[_aligned(u % HT4, DH), :] = (acc * (1.0 / total)).astype(BF16)
                low = jnp.minimum(low, total)
                every = every + acc.reshape(DH // 8, 8, R).sum(axis=0) + total
            p0[...] = pltpu.bitcast(p, U32)
            l0[...] = l
            return low, every

        low, every = lax.fori_loop(
            0, H // HU, fast_heads, (jnp.ones((1, R), F32), jnp.zeros((8, R), F32))
        )

        def safe_heads():
            def safe_tile(tile, _):
                def safe_head(u, _):
                    q = load_q(tile * HT4 + u)

                    def chunk(c, carry):
                        m, l, acc = carry
                        s = _dot(_unpack(kb[_aligned(c, SUB // 2), :]), q)
                        m_new = jnp.maximum(m, jnp.max(s, axis=0, keepdims=True))
                        alpha = jnp.exp2(m - m_new)
                        p = jnp.exp2(s - m_new)
                        l = alpha * l + jnp.sum(p, axis=0, keepdims=True)
                        acc = alpha * acc + _dot(_unpack(vt[_aligned(c, DH // 2), :]), p.astype(BF16))
                        return m_new, l, acc

                    init = (
                        jnp.full((1, R), -jnp.inf, F32),
                        jnp.zeros((1, R), F32),
                        jnp.zeros((DH, R), F32),
                    )
                    _, l, acc = lax.fori_loop(0, NCH, chunk, init)
                    ot[_aligned(u, DH), :] = (acc / l).astype(BF16)

                lax.fori_loop(0, HT4, safe_head, None)
                oa[:, _aligned(tile, 128)] = _pack(ot[...].T)

            lax.fori_loop(0, T, safe_tile, None)

        @pl.when(zero == 0)
        def _():
            oa[:, _tile(T - 1)] = _pack(ot[...].T)
            ok = jnp.where(jnp.logical_and(low >= 1.0, jnp.abs(every) < 3e38), 1.0, 0.0)
            pl.when(jnp.min(ok) < 1.0)(safe_heads)

        first = blk == 0

        def project(src, dst, i, m, emit):
            return [
                piece for t in range(HT) for piece in _strassen(
                    lambda n, t=t: _dot(left_factor(src, dst, i, n), right_factor(m, n, t)),
                    lambda r, c, y, t=t: emit(r * HS, c * HT + t, y),
                )
            ]

        def combine(src, dst, i, r):
            return [
                lambda _, c=c: store_left_factors(src, dst, i, r, c) for c in range(HT // 2)
            ]

        def row_stage(rows, src, dst, i):
            held = []

            def piece(r, token):
                ys, scale = rows(r, token)
                held.append(_lanes([y * scale for y in ys]))
                if len(held) == 2:
                    src[pl.ds((i * SUB + r - 8) // 2, 8), :] = _pack(jnp.concatenate(held, axis=0))
                    held.clear()

            pieces = []
            for r in range(0, HS, 16):
                pieces += [functools.partial(piece, y) for y in (r, r + 8, HS + r, HS + r + 8)]
                if r:
                    pieces += combine(src, dst, i, r - 16)
            return pieces + combine(src, dst, i, HS - 16)

        def out_proj_a(i):
            def emit(r, t, y):
                rows = _aligned((blk * NSUB + i) * 2 + r // HS, HS)
                y = y + xs[t, rows, :]
                x1[t, pl.ds(i * SUB + r, HS), :] = y

            return project(oa, oa_l, i, 0, emit)

        def combine_a(i):
            return [piece for r in range(0, HS, 16) for piece in combine(oa, oa_l, i, r)]

        def norm(i):
            def rows(r, token):
                x = [x1[t, pl.ds(i * SUB + r, 8), :] for t in range(T)]
                return _center([gated(x[0], token)] + x[1:])

            return row_stage(rows, ln, ln_l, i)

        def qkv_proj(i, part):
            def emit(r, t, z):
                if part == 0:
                    lqk[i][t, pl.ds(HALO + r, HS), :] = z
                    return
                refs, t = (lqk, T + t) if part == 1 else (lv, t)
                if i == 0 and r == 0:
                    refs[0][t, 0:HALO, :] = jnp.where(first, z[0:1, :], refs[-1][t, SUB:, :])
                if i + 1 < NSUB and r:
                    refs[i + 1][t, 0:HALO, :] = z[HS - HALO:, :]
                refs[i][t, pl.ds(HALO + r, HS), :] = z

            return project(ln, ln_l, i, part + 1, emit)

        def window(r, w):
            return pl.ds(HALO + r - DIL * w, 8)

        def local_probs(i):
            def piece(r, token):
                scale = gated(np.float32(QSCALE), token)
                q = [lqk[i][t, window(r, 0), :] * scale for t in range(T)]
                z = []
                for w in range(W):
                    y = functools.reduce(jnp.add, [
                        q[t] * lqk[i][T + t, window(r, w), :] for t in range(T)
                    ])
                    y = y + pltpu.roll(y, 2 * H, 1)
                    y = y + pltpu.roll(y, H, 1)
                    if i == 0 and r < DIL * w:
                        pos = row0 + r + lax.broadcasted_iota(jnp.int32, (8, 128), 0)
                        y = jnp.where(pos >= DIL * w, y, MASKED)
                    z.append(y)
                m = functools.reduce(jnp.maximum, z)
                e = [jnp.exp2(y - m) for y in z]
                for w in range(W):
                    lp[i][w, r:r + 8, :] = e[w]
                lp[i][W, r:r + 8, :] = 1.0 / functools.reduce(jnp.add, e)

            return [functools.partial(piece, r) for r in range(0, SUB, 8)]

        def local_values(i):
            def rows(r, token):
                p = [gated(lp[i][w, r:r + 8, :], token) for w in range(W)]
                return [
                    functools.reduce(jnp.add, [p[w] * lv[i][t, window(r, w), :] for w in range(W)])
                    for t in range(T)
                ], lp[i][W, r:r + 8, :]

            return row_stage(rows, ob, ob_l, i)

        def out_proj_b(i):
            def emit(r, t, y):
                rows = pl.ds(i * SUB + r, HS)
                y = y + x1[t, rows, :]
                x1[t, rows, :] = y
                o_ref[rows, _tile(t)] = y.astype(BF16)

            return project(ob, ob_l, i, 4, emit)

        Q, K, V = range(3)
        for piece in combine_a(0):
            piece(None)
        _interleave(out_proj_a(0), (combine_a(1), 0, 25))
        _interleave(out_proj_a(1), (norm(0), 0, 25))
        _interleave(qkv_proj(0, K) + qkv_proj(0, Q), (norm(1), 0, 45))
        _interleave(qkv_proj(1, K) + qkv_proj(1, Q), (local_probs(0), 0, 52))
        _interleave(qkv_proj(0, V), (local_probs(1), 0, 26))
        _interleave(qkv_proj(1, V), (local_values(0), 0, 24))
        _interleave(out_proj_b(0), (local_values(1), 0, 21))
        _interleave(out_proj_b(1), (norm(0), 0, 24))

    @pl.when(step < 2 * NB)
    def _():
        slot = jnp.where(jnp.logical_and(step >= NB, blk < NB - 1), 1, 0)
        part = jnp.where(is_pre, step, 0)

        def cols_in(c, g, token):
            w = pltpu.bitcast(raw[sub(c), _aligned(part * T + g, 128)], U32)
            w = jnp.concatenate([gated(w[:8], token), w[8:]], axis=0).T
            for u in range(4):
                tmp_c[c, pl.ds((4 * g + u) * PAD, DH), :] = w[u * DH:(u + 1) * DH]

        def cols_out(c, g, token):
            w = jnp.concatenate(
                [tmp_c[c, pl.ds(4 * g + u, H, stride=PAD), :] for u in range(4)], axis=0
            )
            w = jnp.concatenate([gated(w[:8], token), w[8:]], axis=0)
            wqkv[part * T + g, _tile(c), :] = w.T

        def wob_tile(i):
            j = jnp.where(part > 0, jnp.minimum(T + 3 * (part - 1) + i, 2 * T - 1), i)
            return j, jnp.where(part > 0, 3 * T + j, j)

        def rows_in(i, n, token):
            w = raw[_aligned(n, 2 * DH), _aligned(wob_tile(i)[1], 128)]
            tmp_r[pl.ds(n * PAD, DH), :] = gated(pltpu.bitcast(w, U32), token)

        def rows_out(i, e, token):
            low = jnp.concatenate([gated(np.uint32(0xFFFF), token)] * 2, axis=0)
            a = tmp_r[pl.ds(e, H // 2, stride=PAD), :]
            b = tmp_r[pl.ds(DH // 2 + e, H // 2, stride=PAD), :]
            even = (a & low) | (b << 16)
            odd = (a >> 16) | (b & ~low)
            wob[wob_tile(i)[0], _aligned(e, H), :] = jnp.concatenate([even, odd], axis=0)

        def place_rows(g, token):
            mask = jnp.concatenate([jnp.logical_and(true, is_pre)] * 2, axis=0)
            x = [
                jnp.where(mask, y, gated(x1[t, _aligned(g, 16), :], token))
                for t, y in enumerate(load_x(blk * (R // 16) + g))
            ]
            for t in range(T):
                xs[t, _aligned(blk * (R // 16) + g, 16), :] = x[t]
            if g < SUB // 16:
                x = [gated(y, token) for y in load_x((blk + 1) % NB * (R // 16) + g)]
            store_norm(g, x)

        def place(i):
            pieces = []
            for r in range(0, HS, 16):
                pieces += [functools.partial(place_rows, (i * SUB + y) // 16) for y in (r, HS + r)]
                pieces += [
                    lambda _, r=r, c=c: store_left_factors(ln, ln_l, i, r, c) for c in range(HT // 2)
                ]
            return pieces

        def project(i, r, size):
            def product(n):
                if n in RIGHT:
                    w = wt_r[pl.ds((RIGHT.index(n) * HWT + r) // 2, size // 2), :]
                else:
                    start = ((n == 5) * HWT + r) // 2
                    w = _lanes([
                        wt[pl.ds(((n == 5) * HT + t) * HWT + start, size // 2), :] for t in range(HT)
                    ])
                return lax.dot_general(
                    _unpack(w), left_factor(ln, ln_l, i, n), NT, preferred_element_type=F32
                )

            held = {}

            def pair(a, b, z):
                if b in held:
                    emit(i, b * HWT + r, _lanes([held.pop(b), z] if a else [z, held.pop(b)]))
                else:
                    held[b] = z

            return _strassen(product, pair)

        def emit(i, r, z):
            nq = min(len(z), D - r)
            rows = pl.ds(pl.multiple_of(blk * (D // 2) + r // 2, 8), nq // 2)
            qt[rows, sub(i)] = _pack(z[:nq])
            if nq == len(z):
                return
            n = blk * NSUB + i
            vt[_aligned(slot * NCH + n, DH // 2), :] = _pack(z[nq + DH:])
            k = z[nq:nq + DH]
            if i == 0:
                mean = jnp.sum(k[:, :128], axis=-1, keepdims=True) * (1.0 / 128)
                kmean[...] = jnp.where(jnp.broadcast_to(blk, (DH, 128)) == 0, mean, kmean[...])
            k = (k - _lanes([kmean[...]] * (SUB // 128))) * QSCALE
            k = jnp.concatenate([k, jnp.zeros((128 - DH, SUB), F32)], axis=0).T
            kb[_aligned(slot * NCH + n, SUB // 2), :] = _pack(k)
            for d in range(DH):
                kv[slot, n, d] = jnp.broadcast_to(k[SUB - VK:, d:d + 1], (VK, 128))

        chunks = [(384, 160), (192, 192), (0, 192)]
        assert sum(chunks[0]) == HWT
        order = [(f, c) for f in (cols_in, cols_out) for c in range(D // SUB)]
        end = 7 * len(chunks) * NSUB
        _interleave(
            [piece for i in range(NSUB) for chunk in chunks for piece in project(i, *chunk)],
            (place(1), 0, end // 2 - 3),
            (place(0), end // 2, end - 2),
            ([functools.partial(f, c, g) for f, c in order for g in range(T)], 0, end - 5),
            ([functools.partial(f, i, n)
              for i in range(3) for f in (rows_in, rows_out) for n in range(16)], 0, end - 1),
        )


@jax.jit
def pallas_interleave_layers__grouped_kv_mqa__sliding_local_dilated__prompt_kernel(
    A_x: jax.Array,
    A_wq: jax.Array,
    A_wk: jax.Array,
    A_wv: jax.Array,
    A_wo: jax.Array,
    B_x: jax.Array,
    B_wqkv: jax.Array,
    B_wo: jax.Array,
):
    del B_x
    _, S, D = A_x.shape
    NB = S // R
    T = D // 128
    vmem = pltpu.VMEM
    left = vmem((NSUB * 5 * SUB // 4, D // 2), U32)
    out = pl.pallas_call(
        _kernel,
        grid=(3 * NB,),
        in_specs=[pl.BlockSpec(memory_space=pl.ANY)] * 7,
        out_specs=pl.BlockSpec((R, D), lambda s: (jnp.maximum(s - 2 * NB, 0), 0)),
        out_shape=jax.ShapeDtypeStruct((S, D), A_x.dtype),
        scratch_shapes=[
            vmem((S, D), BF16),
            vmem((D, 5 * D), BF16),
            vmem((2, DH, D), BF16),
            vmem((T * D, 128), BF16),
            vmem((T * (D // 2 + DH), 128), U32),
            vmem((4 * T, D // 2, 128), U32),
            vmem((2 * T, D // 2, 128), U32),
            vmem((D // SUB, H * PAD, 128), U32),
            vmem((H // 2 * PAD, 128), U32),
            vmem((5 * (D // 2 + DH) // 2, D // 2), U32),
            vmem((5 * 5 * D // 4, D // 2), U32),
            vmem((T, S, 128), F32),
            vmem((T, R, 128), F32),
            vmem((R // 2, D), U32),
            vmem((R // 2, D), U32),
            vmem((R // 2, D), U32),
            left,
            left,
            left,
            vmem((NB * D // 2, R), U32),
            vmem((DH, 128), F32),
            vmem((2 * S // 2, 128), U32),
            vmem((2, S // SUB, DH, VK, 128), F32),
            vmem((2 * S // SUB * DH // 2, SUB), U32),
            vmem((HT4, DH, 8, R), F32),
            vmem((SUB // 2, R), U32),
            vmem((8, R), F32),
            vmem((128, R), BF16),
            vmem((2 * T, HALO + SUB, 128), F32),
            vmem((2 * T, HALO + SUB, 128), F32),
            vmem((T, HALO + SUB, 128), F32),
            vmem((T, HALO + SUB, 128), F32),
            vmem((W + 1, SUB, 128), F32),
            vmem((W + 1, SUB, 128), F32),
            pltpu.SemaphoreType.DMA((S // SUB + 2 * T + 6,)),
        ],
        compiler_params=pltpu.CompilerParams(
            dimension_semantics=("arbitrary",),
            vmem_limit_bytes=120 * 2**20,
        ),
        name="interleave_layers",
    )(A_x.reshape(S, D), A_wq, A_wk.T, A_wv.T, A_wo, B_wqkv, B_wo)
    return out.reshape(1, S, D)
```

```python
import functools
import math

import jax
import jax.numpy as jnp
import numpy as np
from jax import lax
from jax.experimental import pallas as pl
from jax.experimental.pallas import tpu as pltpu

F32 = jnp.float32
BF16 = jnp.bfloat16
U32 = jnp.uint32

H = 32
DH = 32
W = 8
DIL = 2
HALO = 16
EPS = 1e-5
QSCALE = DH ** -0.5 * math.log2(math.e)
MASKED = -1e9 * math.log2(math.e)

R = 512
SUB = 256
NSUB = R // SUB
VK = 16
HPT = 128 // DH
UNITS = DH // 16 * R // 128
PAD = 33

NT = (((1,), (1,)), ((), ()))
HU = 8


def _center(xs):
    inv_d = 1.0 / (128 * len(xs))
    m = jnp.sum(functools.reduce(jnp.add, xs), axis=-1, keepdims=True) * inv_d
    ds = [x - m for x in xs]
    v = jnp.sum(functools.reduce(jnp.add, [d * d for d in ds]), axis=-1, keepdims=True) * inv_d
    return ds, lax.rsqrt(v + EPS)


def _pack(x):
    return pltpu.bitcast(x.astype(BF16), U32)


def _unpack(words):
    return pltpu.bitcast(words, BF16)


def _aligned(index, n):
    start = index * n
    return pl.ds(start if isinstance(start, int) else pl.multiple_of(start, n), n)


def _dot(a, b):
    return jnp.dot(a, b, preferred_element_type=F32)


def _lanes(tiles):
    return jnp.concatenate(tiles, axis=1)


def _tile(t):
    return slice(t * 128, (t + 1) * 128)


LEFT = (1, 2, 5, 6, 7)
RIGHT = (1, 3, 4, 6, 7)


def _left_factors(x11, x12, x21, x22):
    return x11 + x22, x21 + x22, x11 + x12, x21 - x11, x12 - x22


def _right_factors(w11, w12, w21, w22):
    return w11 + w22, w12 - w22, w21 - w11, w11 + w12, w21 + w22


def _strassen(product, emit):
    acc = {}

    def piece(n):
        y = product(n)
        if n == 2:
            acc.update(m2=y)
        elif n == 4:
            emit(1, 0, acc["m2"] + y)
            acc.update(c11=y)
        elif n == 1:
            acc.update(c11=acc["c11"] + y, c22=y - acc["m2"])
        elif n == 7:
            acc.update(c11=acc["c11"] + y)
        elif n == 5:
            emit(0, 0, acc["c11"] - y)
            acc.update(m5=y)
        elif n == 3:
            emit(0, 1, acc["m5"] + y)
            acc.update(c22=acc["c22"] + y)
        else:
            emit(1, 1, acc["c22"] + y)
        return _in_time_order(y)

    return [functools.partial(piece, n) for n in (2, 4, 1, 7, 5, 3, 6)]


def _in_time_order(y):
    return [y[r:r + 8, 0:128] for r in range(0, y.shape[0], 8)]


def _interleave(mxu, *jobs):
    todo = sorted(
        [(start + (stop - start) * i / len(pieces), j, i, piece)
         for j, (pieces, start, stop) in enumerate(jobs) for i, piece in enumerate(pieces)],
        key=lambda item: item[:3],
    )
    for n, piece in enumerate(mxu):
        results = piece()
        while todo and todo[0][0] < n + 1:
            at, _, _, other = todo.pop(0)
            other(results[int((at - n) * len(results))])
    assert not todo


def _kernel(
    x_hbm, wq_hbm, wk_hbm, wv_hbm, woa_hbm, wqkv_hbm, wob_hbm,
    o_ref,
    xin, raw, wkv, woa, wt, wqkv, wob, tmp_c, tmp_r, wt_r, w_r,
    xs, x1, oa, ln, ob, oa_l, ln_l, ob_l,
    qt, kmean, kb, kv, vt, qb, p0, l0, ot,
    lqk0, lqk1, lv0, lv1, lp0, lp1,
    sems,
):
    T, S, _ = xs.shape
    D = T * 128
    NB = S // R
    NCH = S // SUB
    HT, HS, HD = T // 2, SUB // 2, D // 2
    HWT = HD + DH
    lqk, lv, lp = (lqk0, lqk1), (lv0, lv1), (lp0, lp1)
    step = pl.program_id(0)
    is_pre = step < NB
    blk = step % NB
    row0 = pl.multiple_of(blk * R, R)
    zero = jnp.minimum(step, 0)
    true = jnp.broadcast_to(zero, (8, 128)) == 0

    def gated(x, token):
        x = jnp.broadcast_to(x, (8, 128)) if np.ndim(x) == 0 else x
        token = pltpu.bitcast(token, x.dtype)
        return jnp.concatenate(
            [jnp.where(true, x[r:r + 8], token) for r in range(0, x.shape[0], 8)], axis=0
        )

    def sub(i):
        return slice(i * SUB, (i + 1) * SUB)

    def x_copy(i):
        return pltpu.make_async_copy(x_hbm.at[sub(i)], xin.at[sub(i)], sems.at[i])

    def wq_copy(j):
        rows = pl.ds(j * 128, 128)
        return pltpu.make_async_copy(
            wq_hbm.at[rows], raw.at[rows, pl.ds(0, D)], sems.at[NCH + j]
        )

    kv_copies = [
        pltpu.make_async_copy(src, wkv.at[i], sems.at[NCH + T + i])
        for i, src in enumerate([wk_hbm, wv_hbm])
    ]
    raw_copies = [
        pltpu.make_async_copy(src, raw.at[:, pl.ds((i + 1) * D, D)], sems.at[NCH + T + 2 + i])
        for i, src in enumerate([wqkv_hbm.at[:, pl.ds(p * D, D)] for p in range(3)])
    ] + [
        pltpu.make_async_copy(
            wob_hbm.at[:, pl.ds(i * HD, HD)], raw.at[:, pl.ds(4 * D + i * HD, HD)],
            sems.at[NCH + T + 5 + i],
        )
        for i in range(2)
    ]
    woa_copies = [
        pltpu.make_async_copy(
            woa_hbm.at[:, _tile(t)], woa.at[pl.ds(t * D, D)], sems.at[NCH + T + 7 + t]
        )
        for t in range(T)
    ]

    def load_x(g):
        x = xin[_aligned(g, 16), :].astype(F32)
        return [x[:, _tile(t)] for t in range(T)]

    def store_norm(g, x):
        ds, inv = _center(x)
        ln[_aligned(g, 8), :] = _pack(_lanes(ds) * inv)

    def store_left_factors(src, dst, i, r, c):
        ys = _left_factors(*[
            _unpack(src[pl.ds((i * SUB + y) // 2, 8), pl.ds(z + c * 256, 256)]).astype(F32)
            for y in (r, HS + r) for z in (0, HD)
        ])
        for n, y in enumerate(ys):
            dst[pl.ds(((i * 5 + n) * HS + r) // 2, 8), pl.ds(c * 256, 256)] = _pack(y)

    def left_factor(src, dst, i, n):
        if n in LEFT:
            return _unpack(dst[_aligned(i * 5 + LEFT.index(n), HS // 2), :])
        half = n - 3
        return _unpack(src[pl.ds((i * SUB + half * HS) // 2, HS // 2), pl.ds(half * HD, HD)])

    def weight(m, t, half, part=0, parts=1):
        n = HD // parts
        if m == 0:
            return woa[_aligned((2 * t + half) * parts + part, n), :]
        rows = _aligned(half * parts + part, n // 2)
        return _unpack(wob[T + t, rows, :] if m == 4 else wqkv[m * T + t, rows, :])

    def right_factor(m, n, t):
        if n in RIGHT:
            return _unpack(w_r[_aligned(m * 5 + RIGHT.index(n), HD // 2), _tile(t)])
        return weight(m, t + (n == 5) * HT, int(n == 5))

    @pl.when(step == 0)
    def _():
        ahead, n = 4, 2
        x_copy(0).start()
        for j in range(ahead):
            wq_copy(j).start()
        for c in kv_copies:
            c.start()
        lqk1[:, SUB:, :] = jnp.zeros((2 * T, HALO, 128), F32)
        lv1[:, SUB:, :] = jnp.zeros((T, HALO, 128), F32)
        ot[...] = jnp.zeros(ot.shape, BF16)
        kmean[...] = jnp.zeros(kmean.shape, F32)

        @pl.loop(0, T)
        def _(t):
            x1[t] = jnp.zeros((R, 128), F32)

        x_copy(0).wait()

        def first_rows(i, _):
            for u in range(n):
                j = i * n + u
                pl.when(j + ahead < T)(wq_copy(jnp.minimum(j + ahead, T - 1)).start)
                pl.when(j + ahead == T)(x_copy(1).start)
                pl.when(j + ahead == T + 1)(x_copy(2).start)
                wq_copy(j).wait()
            for g in range(SUB // T * n // 16):
                g = i * (SUB // T * n // 16) + g
                store_norm(g, load_x(g))
            for u in range(n):
                j = i * n + u
                wt[pl.ds(pl.multiple_of(j * HWT, 8), HD), :] = _pack(raw[_aligned(j, 128), 0:D].T)

        lax.fori_loop(0, T // n, first_rows, None)
        for i, c in enumerate(kv_copies):
            c.wait()
            for j in range(T):
                wt[pl.ds(j * HWT + (D + i * DH) // 2, DH // 2), :] = pltpu.bitcast(wkv[i, :, _tile(j)], U32)

        for c in range(HT // 2):
            def wt_factors(r, _):
                ys = _right_factors(*[
                    _lanes([
                        _unpack(wt[_aligned(((k + 2 * c + u) * 2 + y) * (HWT // 16) + r, 8), :]).astype(F32)
                        for u in range(2)
                    ])
                    for k in (0, HT) for y in range(2)
                ])
                for j, y in enumerate(ys):
                    wt_r[_aligned(j * (HWT // 16) + r, 8), pl.ds(c * 256, 256)] = _pack(y)

            lax.fori_loop(0, HWT // 16, wt_factors, None, unroll=2)
            for r in range(0, HS, 16):
                store_left_factors(ln, ln_l, 0, r, c)

    for s, waits, starts in ((0, (), (0, 3)), (1, (0, 3), (1, 4)), (2, (1, 4), (2,)), (3, (2,), ())):
        @pl.when(step == s)
        def _():
            for i in range(NSUB * s + 1, min(NSUB * (s + 1) + 1, NCH)):
                x_copy(i).wait()
            for i in waits:
                raw_copies[i].wait()
            for i in range(NSUB * (s + 1) + 1, min(NSUB * (s + 2) + 1, NCH)):
                x_copy(i).start()
            for i in starts:
                raw_copies[i].start()
            if s == NB - 1:
                for c in woa_copies:
                    c.start()

    @pl.when(step == NB)
    def _():
        for c in woa_copies:
            c.wait()

        def w_factors(i, _):
            c, part = i // 16, i % 16
            for m in range(5):
                ys = _right_factors(*[
                    _lanes([weight(m, k + 2 * c + u, half, part, 16).astype(F32) for u in range(2)])
                    for half in range(2) for k in (0, HT)
                ])
                for j, y in enumerate(ys):
                    w_r[_aligned((m * 5 + j) * 16 + part, HD // 32), _aligned(c, 256)] = _pack(y)

        lax.fori_loop(0, HT // 2 * 16, w_factors, None)

    @pl.when(step == 2 * NB)
    def _():
        for ref in (kb, vt):
            half = ref.shape[0] // 2
            n = half // NB * (NB - 1)
            ref[0:n] = ref[half:half + n]

        @pl.loop(0, NSUB * (NB - 1))
        def _(c):
            kv[0, c] = kv[1, c]


    @pl.when(step >= NB)
    def _():
        def q_rows(h):
            return jnp.minimum(blk * H + h, NB * H - 1)

        def load_q(h):
            q = _unpack(qt[_aligned(q_rows(h), DH // 2), :])
            return jnp.concatenate([q, jnp.zeros((128 - DH, R), BF16)], axis=0)

        def spread_q(h, slot, unit, token):
            g, cols = unit // (R // 128), _tile(unit % (R // 128))
            w = qt[_aligned(q_rows(h) * (DH // 16) + g, 8), cols]
            if token is not None:
                w = gated(w, token)
            for odd, y in enumerate((w << 16, w & np.uint32(0xFFFF0000))):
                y = pltpu.bitcast(y, F32)
                for i in range(8):
                    qb[slot, 16 * g + 2 * i + odd, :, cols] = jnp.broadcast_to(y[i:i + 1], (8, 128))

        def scores(q, c):
            return _dot(_unpack(kb[pl.ds(c * SUB // 2, (SUB - VK) // 2), :]), q)

        def probs(s, slot, c, tokens):
            rest = None
            for d in range(DH):
                k = kv[0, c, d]
                if d % 2 == 0:
                    k = gated(k, tokens[d * len(tokens) // DH])
                y = _lanes([k] * (R // 128)) * jnp.concatenate([qb[slot, d]] * (VK // 8), axis=0)
                rest = y if rest is None else rest + y
            p = jnp.exp2(jnp.concatenate([s, rest], axis=0))
            return p.astype(BF16), p.reshape(SUB // 8, 8, R).sum(axis=0)

        @pl.when(blk == 0)
        def _():
            for unit in range(UNITS):
                spread_q(0, 0, unit, None)
            s = scores(load_q(0), 0)
            p, l = probs(s, 0, 0, _in_time_order(s)[:1])
            p0[...] = pltpu.bitcast(p, U32)
            l0[...] = l

        def fast_heads(it, carry):
            low, every = carry
            qs = [load_q(it * HU + u) for u in range(HU + 1)]
            p, l = _unpack(p0[...]), l0[...]
            for u in range(HU):
                acc = None
                for c in range(NCH):
                    v, c2 = u + (c + 1) // NCH, (c + 1) % NCH
                    s = scores(qs[v], c2)
                    pv = _dot(_unpack(vt[_aligned(c, DH // 2), :]), p)
                    acc = pv if acc is None else acc + pv
                    tokens = _in_time_order(s) + _in_time_order(pv)
                    p, l_next = probs(s, v % HPT, c2, tokens)
                    if c2:
                        l = l + l_next
                        units = range(c * UNITS // (NCH - 1), c2 * UNITS // (NCH - 1))
                        for i, unit in enumerate(units):
                            spread_q(it * HU + u + 1, (u + 1) % HPT, unit, tokens[-1 - 15 * i])
                    if u % HPT == 0 and c == 2:
                        w = pltpu.bitcast(ot[...], U32)
                        w = _lanes([gated(w[:, _tile(j)], tokens[0]) for j in range(R // 128)])
                        oa[:, _aligned(((it * HU + u) // HPT + T - 1) % T, 128)] = _pack(_unpack(w).T)
                total = jnp.sum(l, axis=0, keepdims=True)
                l = l_next
                ot[_aligned(u % HPT, DH), :] = (acc * (1.0 / total)).astype(BF16)
                low = jnp.minimum(low, total)
                every = every + acc.reshape(DH // 8, 8, R).sum(axis=0) + total
            p0[...] = pltpu.bitcast(p, U32)
            l0[...] = l
            return low, every

        low, every = lax.fori_loop(
            0, H // HU, fast_heads, (jnp.ones((1, R), F32), jnp.zeros((8, R), F32))
        )

        def safe_heads():
            def safe_tile(tile, _):
                def safe_head(u, _):
                    q = load_q(tile * HPT + u)

                    def chunk(c, carry):
                        m, l, acc = carry
                        s = _dot(_unpack(kb[_aligned(c, SUB // 2), :]), q)
                        m_new = jnp.maximum(m, jnp.max(s, axis=0, keepdims=True))
                        alpha = jnp.exp2(m - m_new)
                        p = jnp.exp2(s - m_new)
                        l = alpha * l + jnp.sum(p, axis=0, keepdims=True)
                        acc = alpha * acc + _dot(_unpack(vt[_aligned(c, DH // 2), :]), p.astype(BF16))
                        return m_new, l, acc

                    init = (
                        jnp.full((1, R), -jnp.inf, F32),
                        jnp.zeros((1, R), F32),
                        jnp.zeros((DH, R), F32),
                    )
                    _, l, acc = lax.fori_loop(0, NCH, chunk, init)
                    ot[_aligned(u, DH), :] = (acc / l).astype(BF16)

                lax.fori_loop(0, HPT, safe_head, None)
                oa[:, _aligned(tile, 128)] = _pack(ot[...].T)

            lax.fori_loop(0, T, safe_tile, None)

        @pl.when(zero == 0)
        def _():
            oa[:, _tile(T - 1)] = _pack(ot[...].T)
            ok = jnp.where(jnp.logical_and(low >= 1.0, jnp.abs(every) < 3e38), 1.0, 0.0)
            pl.when(jnp.min(ok) < 1.0)(safe_heads)

        first = blk == 0

        def project(src, dst, i, m, emit):
            return [
                piece for t in range(HT) for piece in _strassen(
                    lambda n, t=t: _dot(left_factor(src, dst, i, n), right_factor(m, n, t)),
                    lambda r, c, y, t=t: emit(r * HS, c * HT + t, y),
                )
            ]

        def combine(src, dst, i, r):
            return [
                lambda _, c=c: store_left_factors(src, dst, i, r, c) for c in range(HT // 2)
            ]

        def row_stage(rows, src, dst, i):
            held = []

            def piece(r, token):
                ys, scale = rows(r, token)
                held.append(_lanes([y * scale for y in ys]))
                if len(held) == 2:
                    src[pl.ds((i * SUB + r - 8) // 2, 8), :] = _pack(jnp.concatenate(held, axis=0))
                    held.clear()

            pieces = []
            for r in range(0, HS, 16):
                pieces += [functools.partial(piece, y) for y in (r, r + 8, HS + r, HS + r + 8)]
                if r:
                    pieces += combine(src, dst, i, r - 16)
            return pieces + combine(src, dst, i, HS - 16)

        def out_proj_a(i):
            def emit(r, t, y):
                rows = _aligned((blk * NSUB + i) * 2 + r // HS, HS)
                y = y + xs[t, rows, :]
                x1[t, pl.ds(i * SUB + r, HS), :] = y

            return project(oa, oa_l, i, 0, emit)

        def combine_a(i):
            return [piece for r in range(0, HS, 16) for piece in combine(oa, oa_l, i, r)]

        def norm(i):
            def rows(r, token):
                x = [x1[t, pl.ds(i * SUB + r, 8), :] for t in range(T)]
                return _center([gated(x[0], token)] + x[1:])

            return row_stage(rows, ln, ln_l, i)

        def qkv_proj(i, part):
            def emit(r, t, z):
                if part == 0:
                    lqk[i][t, pl.ds(HALO + r, HS), :] = z
                    return
                refs, t = (lqk, T + t) if part == 1 else (lv, t)
                if i == 0 and r == 0:
                    refs[0][t, 0:HALO, :] = jnp.where(first, z[0:1, :], refs[-1][t, SUB:, :])
                if i + 1 < NSUB and r:
                    refs[i + 1][t, 0:HALO, :] = z[HS - HALO:, :]
                refs[i][t, pl.ds(HALO + r, HS), :] = z

            return project(ln, ln_l, i, part + 1, emit)

        def window(r, w):
            return pl.ds(HALO + r - DIL * w, 8)

        def local_probs(i):
            def piece(r, token):
                scale = gated(np.float32(QSCALE), token)
                q = [lqk[i][t, window(r, 0), :] * scale for t in range(T)]
                z = []
                for w in range(W):
                    y = functools.reduce(jnp.add, [
                        q[t] * lqk[i][T + t, window(r, w), :] for t in range(T)
                    ])
                    y = y + pltpu.roll(y, 2 * H, 1)
                    y = y + pltpu.roll(y, H, 1)
                    if i == 0 and r < DIL * w:
                        pos = row0 + r + lax.broadcasted_iota(jnp.int32, (8, 128), 0)
                        y = jnp.where(pos >= DIL * w, y, MASKED)
                    z.append(y)
                m = functools.reduce(jnp.maximum, z)
                e = [jnp.exp2(y - m) for y in z]
                for w in range(W):
                    lp[i][w, r:r + 8, :] = e[w]
                lp[i][W, r:r + 8, :] = 1.0 / functools.reduce(jnp.add, e)

            return [functools.partial(piece, r) for r in range(0, SUB, 8)]

        def local_values(i):
            def rows(r, token):
                p = [gated(lp[i][w, r:r + 8, :], token) for w in range(W)]
                return [
                    functools.reduce(jnp.add, [p[w] * lv[i][t, window(r, w), :] for w in range(W)])
                    for t in range(T)
                ], lp[i][W, r:r + 8, :]

            return row_stage(rows, ob, ob_l, i)

        def out_proj_b(i):
            def emit(r, t, y):
                rows = pl.ds(i * SUB + r, HS)
                y = y + x1[t, rows, :]
                x1[t, rows, :] = y
                o_ref[rows, _tile(t)] = y.astype(BF16)

            return project(ob, ob_l, i, 4, emit)

        Q, K, V = range(3)
        for piece in combine_a(0):
            piece(None)
        _interleave(out_proj_a(0), (combine_a(1), 0, 25))
        _interleave(out_proj_a(1), (norm(0), 0, 25))
        _interleave(qkv_proj(0, K) + qkv_proj(0, Q), (norm(1), 0, 45))
        _interleave(qkv_proj(1, K) + qkv_proj(1, Q), (local_probs(0), 0, 52))
        _interleave(qkv_proj(0, V), (local_probs(1), 0, 26))
        _interleave(qkv_proj(1, V), (local_values(0), 0, 24))
        _interleave(out_proj_b(0), (local_values(1), 0, 20))
        _interleave(out_proj_b(1), (norm(0), 4, 21))

    @pl.when(step < 2 * NB)
    def _():
        slot = jnp.where(jnp.logical_and(step >= NB, blk < NB - 1), 1, 0)
        part = jnp.where(is_pre, step, 0)

        def cols_in(c, g, token):
            w = pltpu.bitcast(raw[sub(c), _aligned(part * T + g, 128)], U32)
            w = jnp.concatenate([gated(w[:8], token), w[8:]], axis=0).T
            for u in range(4):
                tmp_c[c, pl.ds((4 * g + u) * PAD, DH), :] = w[u * DH:(u + 1) * DH]

        def cols_out(c, g, token):
            w = jnp.concatenate(
                [tmp_c[c, pl.ds(4 * g + u, H, stride=PAD), :] for u in range(4)], axis=0
            )
            w = jnp.concatenate([gated(w[:8], token), w[8:]], axis=0)
            wqkv[part * T + g, _tile(c), :] = w.T

        def wob_tile(i):
            j = jnp.where(part > 0, jnp.minimum(T + 3 * (part - 1) + i, 2 * T - 1), i)
            return j, jnp.where(part > 0, 3 * T + j, j)

        def rows_in(i, n, token):
            w = raw[_aligned(n, 2 * DH), _aligned(wob_tile(i)[1], 128)]
            tmp_r[pl.ds(n * PAD, DH), :] = gated(pltpu.bitcast(w, U32), token)

        def rows_out(i, e, token):
            low = jnp.concatenate([gated(np.uint32(0xFFFF), token)] * (H // 16), axis=0)
            a = tmp_r[pl.ds(e, H // 2, stride=PAD), :]
            b = tmp_r[pl.ds(DH // 2 + e, H // 2, stride=PAD), :]
            even = (a & low) | (b << 16)
            odd = (a >> 16) | (b & ~low)
            wob[wob_tile(i)[0], _aligned(e, H), :] = jnp.concatenate([even, odd], axis=0)

        def place_rows(g, token):
            mask = jnp.concatenate([jnp.logical_and(true, is_pre)] * 2, axis=0)
            x = [
                jnp.where(mask, y, gated(x1[t, _aligned(g, 16), :], token))
                for t, y in enumerate(load_x(blk * (R // 16) + g))
            ]
            for t in range(T):
                xs[t, _aligned(blk * (R // 16) + g, 16), :] = x[t]
            if g < SUB // 16:
                x = [gated(y, token) for y in load_x((blk + 1) % NB * (R // 16) + g)]
            store_norm(g, x)

        def place(i):
            pieces = []
            for r in range(0, HS, 16):
                pieces += [functools.partial(place_rows, (i * SUB + y) // 16) for y in (r, HS + r)]
                pieces += [
                    lambda _, r=r, c=c: store_left_factors(ln, ln_l, i, r, c) for c in range(HT // 2)
                ]
            return pieces

        def project(i, r, size):
            def product(n):
                if n in RIGHT:
                    w = wt_r[pl.ds((RIGHT.index(n) * HWT + r) // 2, size // 2), :]
                else:
                    start = ((n == 5) * HWT + r) // 2
                    w = _lanes([
                        wt[pl.ds(((n == 5) * HT + t) * HWT + start, size // 2), :] for t in range(HT)
                    ])
                return lax.dot_general(
                    _unpack(w), left_factor(ln, ln_l, i, n), NT, preferred_element_type=F32
                )

            held = {}

            def pair(a, b, z):
                if b in held:
                    emit(i, b * HWT + r, _lanes([held.pop(b), z] if a else [z, held.pop(b)]))
                else:
                    held[b] = z

            return _strassen(product, pair)

        def emit(i, r, z):
            nq = min(len(z), D - r)
            rows = pl.ds(pl.multiple_of(blk * (D // 2) + r // 2, 8), nq // 2)
            qt[rows, sub(i)] = _pack(z[:nq])
            if nq == len(z):
                return
            n = blk * NSUB + i
            vt[_aligned(slot * NCH + n, DH // 2), :] = _pack(z[nq + DH:])
            k = z[nq:nq + DH]
            if i == 0:
                mean = jnp.sum(k[:, :128], axis=-1, keepdims=True) * (1.0 / 128)
                kmean[...] = jnp.where(jnp.broadcast_to(blk, (DH, 128)) == 0, mean, kmean[...])
            k = (k - _lanes([kmean[...]] * (SUB // 128))) * QSCALE
            k = jnp.concatenate([k, jnp.zeros((128 - DH, SUB), F32)], axis=0).T
            kb[_aligned(slot * NCH + n, SUB // 2), :] = _pack(k)
            for d in range(DH):
                kv[slot, n, d] = jnp.broadcast_to(k[SUB - VK:, d:d + 1], (VK, 128))

        chunks = [(384, 160), (192, 192), (0, 192)]
        assert sum(chunks[0]) == HWT
        order = [(f, c) for f in (cols_in, cols_out) for c in range(D // SUB)]
        end = 7 * len(chunks) * NSUB
        _interleave(
            [piece for i in range(NSUB) for chunk in chunks for piece in project(i, *chunk)],
            (place(1), 0, end // 2 - 3),
            (place(0), end // 2, end - 2),
            ([functools.partial(f, c, g) for f, c in order for g in range(T)], 0, end - 5),
            ([functools.partial(f, i, n)
              for i in range(3) for f in (rows_in, rows_out) for n in range(16)], 0, end - 1),
        )


@jax.jit
def pallas_interleave_layers__grouped_kv_mqa__sliding_local_dilated__prompt_kernel(
    A_x: jax.Array,
    A_wq: jax.Array,
    A_wk: jax.Array,
    A_wv: jax.Array,
    A_wo: jax.Array,
    B_x: jax.Array,
    B_wqkv: jax.Array,
    B_wo: jax.Array,
):
    del B_x
    _, S, D = A_x.shape
    NB = S // R
    T = D // 128
    vmem = pltpu.VMEM
    left = vmem((NSUB * 5 * SUB // 4, D // 2), U32)
    out = pl.pallas_call(
        _kernel,
        grid=(3 * NB,),
        in_specs=[pl.BlockSpec(memory_space=pl.ANY)] * 7,
        out_specs=pl.BlockSpec((R, D), lambda s: (jnp.maximum(s - 2 * NB, 0), 0)),
        out_shape=jax.ShapeDtypeStruct((S, D), A_x.dtype),
        scratch_shapes=[
            vmem((S, D), BF16),
            vmem((D, 5 * D), BF16),
            vmem((2, DH, D), BF16),
            vmem((T * D, 128), BF16),
            vmem((T * (D // 2 + DH), 128), U32),
            vmem((4 * T, D // 2, 128), U32),
            vmem((2 * T, D // 2, 128), U32),
            vmem((D // SUB, (H + 1) * PAD, 128), U32),
            vmem(((H // 2 + 1) * PAD + 7, 128), U32),
            vmem((5 * (D // 2 + DH) // 2, D // 2), U32),
            vmem((5 * 5 * D // 4, D // 2), U32),
            vmem((T, S, 128), F32),
            vmem((T, R, 128), F32),
            vmem((R // 2, D), U32),
            vmem((R // 2, D), U32),
            vmem((R // 2, D), U32),
            left,
            left,
            left,
            vmem((NB * D // 2, R), U32),
            vmem((DH, 128), F32),
            vmem((2 * S // 2, 128), U32),
            vmem((2, S // SUB, DH, VK, 128), F32),
            vmem((2 * S // SUB * DH // 2, SUB), U32),
            vmem((HPT, DH, 8, R), F32),
            vmem((SUB // 2, R), U32),
            vmem((8, R), F32),
            vmem((128, R), BF16),
            vmem((2 * T, HALO + SUB, 128), F32),
            vmem((2 * T, HALO + SUB, 128), F32),
            vmem((T, HALO + SUB, 128), F32),
            vmem((T, HALO + SUB, 128), F32),
            vmem((W + 1, SUB, 128), F32),
            vmem((W + 1, SUB, 128), F32),
            pltpu.SemaphoreType.DMA((S // SUB + 2 * T + 7,)),
        ],
        compiler_params=pltpu.CompilerParams(
            dimension_semantics=("arbitrary",),
            vmem_limit_bytes=110 * 2**20,
        ),
        name="interleave_layers",
    )(A_x.reshape(S, D), A_wq, A_wk.T, A_wv.T, A_wo, B_wqkv, B_wo)
    return out.reshape(1, S, D)
```
